```python
import os as _os
_os.environ.setdefault('JAX_PLATFORMS', 'cpu')
import jax
import jax.numpy as jnp

def _softmax(x, axis=-1):
    return jax.nn.softmax(x, axis=axis)

def _gelu(x):
    return jax.nn.gelu(x, approximate=True)

def _silu(x):
    return jax.nn.silu(x)

def _sigmoid(x):
    return jax.nn.sigmoid(x)

def _layernorm(x, axis=-1, eps=1e-05):
    m = jnp.mean(x, axis=axis, keepdims=True)
    v = jnp.var(x, axis=axis, keepdims=True)
    return (x - m) / jnp.sqrt(v + eps)

def _scatter_add(tgt, idx, src, axis=0):
    return tgt.at[idx].add(src)

def _segment_sum(src, seg, n):
    return jax.ops.segment_sum(src, seg, n)

class _Rng:

    def __init__(self, key):
        self._k = key

    def _next(self):
        self._k, sub = jax.random.split(self._k)
        return sub

    def normal(self, shape):
        return jax.random.normal(self._next(), shape, dtype=jnp.bfloat16)

    def randint(self, lo, hi, shape):
        return jax.random.randint(self._next(), shape, lo, hi, dtype=jnp.int32)

    def uniform(self, shape, lo=0.0, hi=1.0):
        return jax.random.uniform(self._next(), shape, jnp.bfloat16, lo, hi)

    def permutation(self, n):
        return jax.random.permutation(self._next(), n)
kernel_name = 'adaLN_cond__mha_block__geglu_ffn__prompt'

def setup_inputs():
    _rng = _Rng(jax.random.key(int.from_bytes(__import__("os").urandom(4), "little")))
    _w = lambda a: (lambda t: t.astype(jnp.bfloat16) if jnp.issubdtype(t.dtype, jnp.floating) else t)(jnp.asarray(a))

    def _A_setup():
        B, S, D, H = (1, 2048, 640, 32)
        return {'x': _w((lambda *s: _rng.normal(s) * 0.05)(B, S, D)), 'wqkv': _w((lambda *s: _rng.normal(s) * 0.05)(D, 3 * D)), 'wo': _w((lambda *s: _rng.normal(s) * 0.05)(D, D))}
    _A_in = _A_setup()

    def _B_setup():
        B, S, D, F = (1, 2048, 640, 1728)
        return {'x': _w((lambda *s: _rng.normal(s) * 0.05)(B, S, D)), 'w_gate': _w((lambda *s: _rng.normal(s) * 0.05)(D, F)), 'w_up': _w((lambda *s: _rng.normal(s) * 0.05)(D, F)), 'w_down': _w((lambda *s: _rng.normal(s) * 0.05)(F, D))}
    _B_in = _B_setup()
    return {'A_x': _A_in['x'], 'A_wqkv': _A_in['wqkv'], 'A_wo': _A_in['wo'], 'B_x': _B_in['x'], 'B_w_gate': _B_in['w_gate'], 'B_w_up': _B_in['w_up'], 'B_w_down': _B_in['w_down'], 'c': _w((lambda *s: _rng.normal(s) * 0.05)(1, 640) * 8.0), 'w_mod': _w((lambda *s: _rng.normal(s) * 0.05)(640, 6 * 640) * 640 ** (-0.5) * 8.0)}

def reference(A_x, A_wqkv, A_wo, B_x, B_w_gate, B_w_up, B_w_down, c, w_mod):

    def _A_ref(x, wqkv, wo):
        B, S, D = x.shape
        H = 32
        Dh = D // H
        qkv = (lambda x, *d: x.transpose(*d))((x @ wqkv).reshape(B, S, 3, H, Dh), 2, 0, 3, 1, 4)
        q, k, v = (qkv[0], qkv[1], qkv[2])
        scores = jnp.einsum('bhqd,bhkd->bhqk', q, k) * Dh ** (-0.5)
        p = _softmax(scores, axis=-1)
        o = jnp.einsum('bhqk,bhkd->bhqd', p, v)
        return (lambda x, *d: x.transpose(*d))(o, 0, 2, 1, 3).reshape(B, S, D) @ wo

    def _B_ref(x, w_gate, w_up, w_down):
        return _gelu(x @ w_gate) * (x @ w_up) @ w_down
    x = A_x
    mod = (_silu(c) @ w_mod).reshape(c.shape[0], 6, 1, -1)
    sa, ca, ga, sb, cb, gb = (mod[:, 0].copy(), mod[:, 1].copy(), mod[:, 2].copy(), mod[:, 3].copy(), mod[:, 4].copy(), mod[:, 5].copy())
    h = _layernorm(x, axis=-1) * (1 + ca) + sa
    x = x + ga * _A_ref(h, A_wqkv, A_wo)
    h = _layernorm(x, axis=-1) * (1 + cb) + sb
    x = x + gb * _B_ref(h, B_w_gate, B_w_up, B_w_down)
    return x
```

```python
import functools
import math

import jax
import jax.numpy as jnp
from jax import lax
import jax.experimental.pallas as pl
import jax.experimental.pallas.tpu as pltpu

S, D, H, F = 2048, 640, 32, 1728
DH = D // H
VR = 24
NWIN = 9
EPS = 1e-5
f32, bf16, u32 = jnp.float32, jnp.bfloat16, jnp.uint32

NN = (((1,), (0,)), ((), ()))
NT = (((1,), (1,)), ((), ()))
TN = (((0,), (0,)), ((), ()))


def _dot(a, b, dims=NN):
    return lax.dot_general(a, b, dims, preferred_element_type=f32)


def _layernorm(x):
    mean = jnp.mean(x, axis=-1, keepdims=True)
    xc = x - mean
    var = jnp.mean(xc * xc, axis=-1, keepdims=True)
    return xc * lax.rsqrt(var + EPS)


def _make_kernel(TA, QB, KC, SKEW, TB):
    NQB = S // QB
    NKC = S // KC
    FM = (F // 128) * 128
    FR = F - FM

    def kernel(x_hbm, wqkv_hbm, wo_hbm, wgt_hbm, wut_hbm, wd_hbm, c_ref, wmod_hbm,
               out_hbm,
               x_v, wqkv_v, wo_v, wgu_v, wd_v, wmod_v, wqvt_v,
               k_s, q_s, v_s, ot_s, s_a, s_b, out_v, sem_in, sem_x, sem_out):
        def cp(src, dst, i):
            return pltpu.make_async_copy(src, dst, sem_in.at[i])
        cp_mod_a = cp(wmod_hbm.at[:, pl.ds(0, 2 * D)], wmod_v.at[:, pl.ds(0, 2 * D)], 0)
        cp_wqkv = cp(wqkv_hbm, wqkv_v, 1)
        late = [
            cp(wmod_hbm.at[:, pl.ds(2 * D, 4 * D)], wmod_v.at[:, pl.ds(2 * D, 4 * D)], 2),
            cp(wo_hbm, wo_v, 3),
            cp(wgt_hbm.at[pl.ds(0, FM)], wgu_v.at[pl.ds(0, FM)], 4),
            cp(wut_hbm.at[pl.ds(0, FM)], wgu_v.at[pl.ds(FM, FM)], 5),
            cp(wgt_hbm.at[pl.ds(FM, FR)], wgu_v.at[pl.ds(2 * FM, FR)], 6),
            cp(wut_hbm.at[pl.ds(FM, FR)], wgu_v.at[pl.ds(2 * FM + FR, FR)], 7),
            cp(wd_hbm, wd_v, 8),
        ]
        cp_x = [pltpu.make_async_copy(x_hbm.at[pl.ds(i * TA, TA)], x_v.at[pl.ds(i * TA, TA)], sem_x.at[i])
                for i in range(S // TA)]
        cp_mod_a.start()
        cp_x[0].start()
        cp_wqkv.start()
        for d in cp_x[1:]:
            d.start()

        s_b[...] = jnp.zeros(s_b.shape, f32)

        cf = c_ref[...].astype(f32)
        sc = jnp.broadcast_to(cf * jax.nn.sigmoid(cf), (16, D)).astype(bf16)
        cp_mod_a.wait()
        mod_a = _dot(sc, wmod_v[:, pl.ds(0, 2 * D)])[0:1]
        sa, ca1 = mod_a[:, :D], 1.0 + mod_a[:, D:]

        cp_wqkv.wait()
        wqvt_v[pl.ds(0, D), :] = wqkv_v[:, pl.ds(0, D)].T
        wqvt_v[pl.ds(D, D), :] = wqkv_v[:, pl.ds(2 * D, D)].T

        qscale = DH ** -0.5 * math.log2(math.e)
        for i in range(S // TA):
            cp_x[i].wait()
            if i == S // TA - 1:
                for d in late:
                    d.start()
            r0 = i * TA
            h = (_layernorm(x_v[pl.ds(r0, TA), :].astype(f32)) * ca1 + sa).astype(bf16)
            k = _dot(h, wqkv_v[:, pl.ds(D, D)])
            kw = [pltpu.bitcast(k[:, t * 128:(t + 1) * 128].astype(bf16), u32) for t in range(5)]
            hi = lax.broadcasted_iota(jnp.int32, kw[0].shape, 1) >= 64
            for t in range(5):
                k_s[t, pl.ds(r0 // 2, TA // 2), :] = kw[t]
            for t in range(4):
                k_s[5 + t, pl.ds(r0 // 2, TA // 2), :] = jnp.where(hi, kw[t], kw[t + 1])
            qt = _dot(wqvt_v[pl.ds(0, D), :], h, NT) * qscale
            qw = pltpu.bitcast(qt.astype(bf16), u32)
            for t in range(5):
                q_s[t, :, pl.ds(r0, TA)] = qw[t * 64:(t + 1) * 64]
            for t in range(4):
                q_s[5 + t, pl.ds(0, 32), pl.ds(r0, TA)] = qw[(t + 1) * 64:(t + 1) * 64 + 32]
                q_s[5 + t, pl.ds(32, 32), pl.ds(r0, TA)] = qw[t * 64 + 32:(t + 1) * 64]
            vt = _dot(wqvt_v[pl.ds(D, D), :], h, NT)
            lo = lax.broadcasted_iota(jnp.int32, (8, TA), 0) < 4
            for j in range(H // 2):
                b = 40 * j
                mid = vt[b + 16:b + 24]
                v_s[2 * j, pl.ds(0, 16), pl.ds(r0, TA)] = vt[b:b + 16]
                v_s[2 * j, pl.ds(16, 8), pl.ds(r0, TA)] = jnp.where(lo, mid, 1.0)
                v_s[2 * j + 1, pl.ds(0, 8), pl.ds(r0, TA)] = jnp.where(lo, 1.0, mid)
                v_s[2 * j + 1, pl.ds(8, 16), pl.ds(r0, TA)] = vt[b + 24:b + 40]

        def pv_chunk(cur, m_cur, hv, j, acc):
            p = jnp.exp2(cur[pl.ds(j * KC, KC), :] - m_cur)
            return acc + _dot(v_s[hv, :, pl.ds(j * KC, KC)], p)

        def head(hd, m):
            lo_f = hd * DH
            t0 = lo_f >> 7
            t1 = (lo_f + DH - 1) >> 7
            win = jnp.where(t0 == t1, t0, 5 + t0)
            rel = (lax.broadcasted_iota(jnp.int32, (64, QB), 0) - ((lo_f & 127) >> 1)) & 63
            qmask = rel < DH // 2
            for t in range(NQB):
                nxt, cur = (s_a, s_b) if t % 2 == 0 else (s_b, s_a)
                if t == 0:
                    hv = jnp.maximum(hd - 1, 0)
                    ho = jnp.where(hd == 0, H, hd - 1)
                    po = (NQB - 1) * QB
                else:
                    hv, ho, po = hd, hd, (t - 1) * QB
                qt = pltpu.bitcast(jnp.where(qmask, q_s[win, :, pl.ds(t * QB, QB)], u32(0)), bf16)
                acc = jnp.zeros((VR, QB), f32)
                mx = jnp.full((8, QB), -jnp.inf, f32)
                for j in range(NKC + SKEW):
                    if j < NKC:
                        s = _dot(pltpu.bitcast(k_s[win, pl.ds(j * KC // 2, KC // 2), :], bf16), qt)
                        nxt[pl.ds(j * KC, KC), :] = s
                        mx = jnp.maximum(mx, jnp.max(s.reshape(KC // 8, 8, QB), axis=0))
                    if j >= SKEW:
                        acc = pv_chunk(cur, m, hv, j - SKEW, acc)
                ot_s[ho, :, pl.ds(po, QB)] = acc
                m = jnp.max(mx, axis=0, keepdims=True)
            return m

        m = lax.fori_loop(0, H, head, jnp.zeros((1, QB), f32))
        acc = jnp.zeros((VR, QB), f32)
        for j in range(NKC):
            acc = pv_chunk(s_b, m, H - 1, j, acc)
        ot_s[H - 1, :, pl.ds((NQB - 1) * QB, QB)] = acc

        for d in late:
            d.wait()
        mod_b = _dot(sc, wmod_v[:, pl.ds(2 * D, 4 * D)])[0:1]
        ga, sb, cb1, gb = mod_b[:, :D], mod_b[:, D:2 * D], 1.0 + mod_b[:, 2 * D:3 * D], mod_b[:, 3 * D:]
        c0 = math.sqrt(2.0 / math.pi)
        c1 = c0 * 0.044715

        def geglu(g, u):
            return (0.5 * g * u) * (1.0 + jnp.tanh(g * (c0 + c1 * (g * g))))

        def out_cp(i):
            r0 = pl.multiple_of(i * TB, TB)
            return pltpu.make_async_copy(out_v.at[pl.ds(r0, TB)], out_hbm.at[pl.ds(r0, TB)], sem_out.at[i])

        def block(i, carry):
            r0 = pl.multiple_of(i * TB, TB)
            lo = lax.broadcasted_iota(jnp.int32, (8, TB), 0) < 4
            rows = []
            for j in range(H // 2):
                e = ot_s[2 * j, :, pl.ds(r0, TB)]
                o = ot_s[2 * j + 1, :, pl.ds(r0, TB)]
                re = 1.0 / e[20:21]
                ro = 1.0 / o[0:1]
                rows += [e[0:16] * re, jnp.where(lo, e[16:24] * re, o[0:8] * ro), o[8:24] * ro]
            ot = jnp.concatenate(rows, axis=0).astype(bf16)
            x1 = x_v[pl.ds(r0, TB), :].astype(f32) + ga * _dot(ot, wo_v[...], TN)
            h2 = (_layernorm(x1) * cb1 + sb).astype(bf16)
            g = _dot(h2, wgu_v[pl.ds(0, FM), :], NT)
            u = _dot(h2, wgu_v[pl.ds(FM, FM), :], NT)
            gu = _dot(h2, wgu_v[pl.ds(2 * FM, 2 * FR), :], NT)
            a_main = geglu(g, u).astype(bf16)
            a_rest = geglu(gu, pltpu.roll(gu, FR, 1))[:, :FR].astype(bf16)
            y = _dot(a_main, wd_v[pl.ds(0, FM), :]) + _dot(a_rest, wd_v[pl.ds(FM, FR), :])
            out_v[pl.ds(r0, TB), :] = (x1 + gb * y).astype(bf16)
            out_cp(i).start()
            return carry

        lax.fori_loop(0, S // TB, block, 0)
        for i in range(S // TB):
            out_cp(i).wait()

    return kernel


def build(TA=512, QB=512, KC=128, SKEW=1, TB=512):
    def fn(A_x, A_wqkv, A_wo, B_x, B_w_gate, B_w_up, B_w_down, c, w_mod):
        hbm = pl.BlockSpec(memory_space=pltpu.MemorySpace.HBM)
        vmem = pl.BlockSpec(memory_space=pltpu.MemorySpace.VMEM)
        out = pl.pallas_call(
            _make_kernel(TA, QB, KC, SKEW, TB),
            out_shape=jax.ShapeDtypeStruct((S, D), bf16),
            in_specs=[hbm, hbm, hbm, hbm, hbm, hbm, vmem, hbm],
            out_specs=hbm,
            scratch_shapes=[
                pltpu.VMEM((S, D), bf16),
                pltpu.VMEM((D, 3 * D), bf16),
                pltpu.VMEM((D, D), bf16),
                pltpu.VMEM((2 * F, D), bf16),
                pltpu.VMEM((F, D), bf16),
                pltpu.VMEM((D, 6 * D), bf16),
                pltpu.VMEM((2 * D, D), bf16),
                pltpu.VMEM((NWIN, S // 2, 128), u32),
                pltpu.VMEM((NWIN, 64, S), u32),
                pltpu.VMEM((H, VR, S), f32),
                pltpu.VMEM((H + 1, VR, S), f32),
                pltpu.VMEM((S, QB), f32),
                pltpu.VMEM((S, QB), f32),
                pltpu.VMEM((S, D), bf16),
                pltpu.SemaphoreType.DMA((9,)),
                pltpu.SemaphoreType.DMA((S // TA,)),
                pltpu.SemaphoreType.DMA((S // TB,)),
            ],
            compiler_params=pltpu.CompilerParams(vmem_limit_bytes=120 * 1024 * 1024),
            name="adaln_block",
        )(A_x.reshape(S, D), A_wqkv, A_wo, B_w_gate.T, B_w_up.T, B_w_down, c, w_mod)
        return out.reshape(1, S, D)
    return fn


@jax.jit
def pallas_adaLN_cond__mha_block__geglu_ffn__prompt_kernel(
    A_x: jax.Array,
    A_wqkv: jax.Array,
    A_wo: jax.Array,
    B_x: jax.Array,
    B_w_gate: jax.Array,
    B_w_up: jax.Array,
    B_w_down: jax.Array,
    c: jax.Array,
    w_mod: jax.Array,
):
    return build()(A_x, A_wqkv, A_wo, B_x, B_w_gate, B_w_up, B_w_down, c, w_mod)
```

```python
import contextlib
import math

import jax
import jax.numpy as jnp
from jax import lax
import jax.experimental.pallas as pl
import jax.experimental.pallas.tpu as pltpu

S, D, H, F = 2048, 640, 32, 1728
DH = D // H
NP = H // 2
PW = 2 * DH
VR = 24
TA = 512
QB, KC = 512, 128
NV = 16
TB = 256
HB = TB // 2
LR = 32
NQB, NKC, LT = S // QB, S // KC, QB // 128
EPS = 1e-5
f32, bf16, i32 = jnp.float32, jnp.bfloat16, jnp.int32

NN = (((1,), (0,)), ((), ()))
NT = (((1,), (1,)), ((), ()))


def _dot(a, b, dims=NN):
    return lax.dot_general(a, b, dims, preferred_element_type=f32)


def _layernorm(x):
    mean = jnp.mean(x, axis=-1, keepdims=True)
    xc = x - mean
    var = jnp.mean(xc * xc, axis=-1, keepdims=True)
    return xc * lax.rsqrt(var + EPS)


def _geglu_x2(g, u):
    c0 = math.sqrt(2.0 / math.pi)
    return (g * u) * (1.0 + jnp.tanh(g * (c0 + (c0 * 0.044715) * (g * g))))


def _after(val, ref, zero, row=0):
    lead = (0,) * (len(ref.shape) - 2)
    w = pltpu.bitcast(ref[lead + (pl.ds(pl.multiple_of(zero * 8, 8), 8), pl.ds(0, 128))], i32) & zero
    head = pltpu.bitcast(pltpu.bitcast(val[row:row + 8, :128], i32) | w, f32)
    mid = jnp.concatenate([head, val[row:row + 8, 128:]], axis=1)
    return jnp.concatenate(([val[:row]] if row else []) + [mid, val[row + 8:]], axis=0)


class _Lin(dict):
    def __add__(self, other):
        out = _Lin(self)
        for key, c in other.items():
            out[key] = out.get(key, 0) + c
        return _Lin({key: c for key, c in out.items() if c})

    def __neg__(self):
        return _Lin({key: -c for key, c in self.items()})

    def __sub__(self, other):
        return self + (-other)

    def times(self, c):
        return self if c > 0 else -self


def _hopcroft_kerr(kinds, helpers):
    lhs, out = [], []

    def product(a, b):
        lhs.append(a)
        out.append(b)
        return _Lin({len(lhs) - 1: 1})

    def node(ca, cb, kind, diag=None):
        f = lambda x: _Lin({(k, x % 3): c for k, c in ca.items()})
        g = lambda x: _Lin({(k, x % 3): c for k, c in cb.items()})
        diag = diag or (product(f(kind + 1), g(kind + 2)), product(f(kind + 2), g(kind + 1)))
        return dict(f=f, g=g, kind=kind, diag=diag, ca=ca, cb=cb)

    def pair(p, q):
        if (p['kind'] - q['kind']) % 3 != 1:
            qp, pq, both = pair(q, p)
            return pq, qp, both
        x = q['kind']
        m1 = product(p['f'](x) + q['f'](x + 1), q['g'](x + 1) - p['g'](x))
        m6 = product(q['f'](x) - p['f'](x), q['g'](x + 1) + p['g'](x + 1))
        m7 = product(q['f'](x + 1) - p['f'](x + 1), q['g'](x) + p['g'](x))
        both = node(q['ca'] - p['ca'], p['cb'] + q['cb'], (x + 2) % 3, (m6, m7))
        return m1 + q['diag'][0] - p['diag'][0] + m7, m1 + q['diag'][1] - p['diag'][1] + m6, both

    n = len(kinds)
    nodes = [node(_Lin({i: 1}), _Lin({i: 1}), kinds[i]) for i in range(n)]
    use = {(i, i): nodes[i]['diag'][0] - nodes[i]['diag'][1] for i in range(n)}
    merged = {}
    for i in range(n):
        for j in range(i + 1, n):
            if kinds[i] != kinds[j]:
                use[i, j], use[j, i], merged[i, j] = pair(nodes[i], nodes[j])
    for i, j, h in helpers:
        v = merged[min(i, h), max(i, h)]
        vj, jv, _ = pair(v, nodes[j])
        use[i, j] = (vj - use[h, j].times(v['ca'][h])).times(v['ca'][i])
        use[j, i] = (jv - use[j, h].times(v['cb'][h])).times(v['cb'][i])
    rhs = [_Lin({kj: lin[r] for kj, lin in use.items() if r in lin}) for r in range(len(lhs))]
    return list(zip(lhs, rhs, out))


_SCHEME = _hopcroft_kerr((0, 0, 1, 1, 2), ((0, 1, 2), (2, 3, 0)))
_SUMMED = [r for r, (_, rhs, _) in enumerate(_SCHEME) if len(rhs) > 1]
_GROUPS = ([[r, r + 1] for r in range(0, 10, 2)]
           + [[10 + 3 * x, 11 + 3 * x, 12 + 3 * x] for x in (2, 5, 6, 7, 3, 8, 4, 9, 1, 0)])


def _signed_sum(terms):
    terms = sorted(terms, key=lambda t: -t[0])
    sign, acc = terms[0]
    for c, v in terms[1:]:
        acc = acc + v if c == sign else acc - v
    return sign, acc


def _weight_sums(block):
    w = {(k, j): block(k, j).astype(f32) for k in range(5) for j in range(5)}
    return [_signed_sum([(c, w[kj]) for kj, c in _SCHEME[r][1].items()])[1] for r in _SUMMED]


def _fast_lhs(a, dtype):
    f = {}
    for k in range(5):
        f[k, 0], f[k, 1], f[k, 2] = (1, a[0][k]), (1, a[1][k]), (-1, a[0][k] + a[1][k])
    out = []
    for lhs, _, _ in _SCHEME:
        sign, v = _signed_sum([(c * f[kx][0], f[kx][1]) for kx, c in lhs.items()])
        out.append((sign, v.astype(dtype)))
    return out


def _fast_matmul(lhs, block, sums, dims):
    t = {}
    for group in _GROUPS:
        new = {}
        for r in group:
            (sign, a), (_, rhs, out) = lhs[r], _SCHEME[r]
            w = sums(_SUMMED.index(r)) if r in _SUMMED else block(*next(iter(rhs)))
            m = _dot(a, w, dims)
            for jx, c in out.items():
                new.setdefault(jx, []).append((c * sign * max(rhs.values()), m))
        for jx, terms in new.items():
            t[jx] = _signed_sum([_signed_sum(terms)] + ([t[jx]] if jx in t else []))

    def diff(p, q):
        sign, v = _signed_sum([p, (-q[0], q[1])])
        return v if sign > 0 else -v
    return [[diff(t[j, 1], t[j, 2]) for j in range(5)], [diff(t[j, 2], t[j, 0]) for j in range(5)]]


def _make_kernel(SC, CUT, R, R0, ORD, LATE, LAG):
    scope = jax.named_scope if SC else (lambda n: contextlib.nullcontext())

    def kernel(x_hbm, wqkv_hbm, wo_hbm, wgt_hbm, wut_hbm, wd_hbm, c_hbm, wmod_hbm,
               out_hbm,
               c_v, x_v, wqkv_v, wo_v, wup_v, wd_v, wmod_v, ws_s, h_s, qf_s, h2a_s, h2b_s,
               k_s, q_s, v_s, kb0_s, kb1_s, ot_s, o_s, out_v, sem_in, sem_out):
        copies = []

        def fetch(src, dst):
            copies.append(pltpu.make_async_copy(src, dst, sem_in.at[len(copies)]))
            return copies[-1]

        def wait(*group):
            for d in group:
                d.wait()

        rows = lambda ref, a, n: ref.at[pl.ds(a, n)]
        cols = lambda ref, a, n: ref.at[:, pl.ds(a, n)]
        fetch_x = lambda i: fetch(rows(x_hbm, i * TA, TA), rows(x_v, i * TA, TA))
        fetch_cols = lambda src, dst, a, n: fetch(cols(src, a, n), cols(dst, a, n))
        halves = ((0, 384), (384, 256))

        cp_c = fetch(c_hbm, cols(c_v, 0, D))
        cp_x0 = fetch_x(0)
        cp_first = [(fetch_cols(wmod_hbm, wmod_v, a, n), fetch_cols(wmod_hbm, wmod_v, D + a, n),
                     fetch(wqkv_hbm.at[pl.ds(a, n), pl.ds(0, D)], wqkv_v.at[pl.ds(a, n), pl.ds(0, D)]))
                    for a, n in halves]
        cp_a = [fetch_cols(wqkv_hbm, wqkv_v, D, D), fetch_x(1)]
        cp_b = [fetch_cols(wqkv_hbm, wqkv_v, 2 * D, D), fetch_x(2), fetch_x(3),
                fetch(rows(wgt_hbm, 0, 2 * D), rows(wup_v, 0, 2 * D))]
        cp_c2 = [fetch(rows(wut_hbm, 0, 2 * D), rows(wup_v, 2 * D, 2 * D)), fetch(wd_hbm, wd_v),
                 fetch_cols(wmod_hbm, wmod_v, 2 * D, 4 * D)]
        for j in range(5):
            cp_c2.append(fetch(rows(wgt_hbm, 2 * D + 64 * j, 64), rows(wup_v, 4 * D + 128 * j + 64 * (j % 2), 64)))
            cp_c2.append(fetch(rows(wut_hbm, 2 * D + 64 * j, 64), rows(wup_v, 4 * D + 128 * j + 64 * (1 - j % 2), 64)))
        cp_d = [fetch(wo_hbm, wo_v), fetch(rows(wgt_hbm, F - 128, 128), rows(wup_v, 5 * D, 128)),
                fetch(rows(wut_hbm, F - 128, 128), rows(wup_v, 5 * D + 128, 128))]

        with scope('p0'):
            for d in copies:
                d.start()
            wait(cp_c)
            cf = c_v[:, pl.ds(0, D)].astype(f32)
            gate = jax.nn.sigmoid(cf)
            sc = jnp.broadcast_to(cf * gate, (16, D)).astype(bf16)
            zero0 = jnp.max(jnp.where(gate[:, :128] > 2.0, 1, 0))
            wait(cp_x0)
            for r in range(0, TA, 64):
                h_s[pl.ds(r, 64), :] = _layernorm(x_v[pl.ds(r, 64), :].astype(f32))
            sa, ca1 = [], []
            for (a, n), (d_shift, d_scale, d_wq) in zip(halves, cp_first):
                wait(d_shift, d_scale)
                sa.append(_dot(sc, wmod_v[:, pl.ds(a, n)])[0:1])
                ca1.append(1.0 + _dot(sc, wmod_v[:, pl.ds(D + a, n)])[0:1])
                for r in range(0, TA, LR):
                    h_s[pl.ds(r, LR), pl.ds(a, n)] = h_s[pl.ds(r, LR), pl.ds(a, n)] * ca1[-1] + sa[-1]
                wait(d_wq)
                if a == 0:
                    qf_s[zero0] = _dot(h_s[pl.ds(0, TA), pl.ds(a, n)], wqkv_v[pl.ds(a, n), pl.ds(0, D)])
            sa, ca1 = jnp.concatenate(sa, axis=1), jnp.concatenate(ca1, axis=1)

        v_peaks = []

        def ln_block(i):
            for r in range(i * TA, (i + 1) * TA, LR):
                h_s[pl.ds(r, LR), :] = _layernorm(x_v[pl.ds(r, LR), :].astype(f32)) * ca1 + sa

        def project(m, i, jobs=(), after_k=False):
            h = h_s[pl.ds(i * TA, TA), :]
            jobs = list(jobs)
            per = -(-len(jobs) // (5 * TA // 64))
            parts = []
            for c0 in range(0, D, 128):
                lhs = _after(h, k_s, zero0, 8) if after_k and c0 >= 256 else h
                for row in range(0, TA, 64):
                    if jobs:
                        for job in jobs[:per]:
                            job()
                        jobs = jobs[per:]
                        lhs = _after(lhs, ws_s, zero0, row)
                parts.append(_dot(lhs, wqkv_v[:, pl.ds(m * D + c0, 128)]))
            return jnp.concatenate(parts, axis=1)

        def store_q(i, q):
            qt = (q * (DH ** -0.5 * math.log2(math.e))).T
            for j in range(NP):
                q_s[j, :, pl.ds(i * TA, TA)] = qt[j * PW:(j + 1) * PW]

        def store_k(i, k):
            hi = lax.broadcasted_iota(i32, (TA, 128), 1) >= 64
            for j in range(NP):
                t, o = divmod(j * PW, 128)
                w = k[:, t * 128:(t + 1) * 128]
                if o + PW > 128:
                    w = jnp.where(hi, w, k[:, (t + 1) * 128:(t + 2) * 128])
                k_s[j, pl.ds(i * TA, TA), :] = pltpu.roll(w, 128 - o, 1) if o else w

        def store_v(i, v):
            vt = v.T
            v_peaks.append(jnp.max(jnp.abs(vt).reshape(D // 8, 8, TA), axis=0))
            lo = lax.broadcasted_iota(i32, (8, TA), 0) < 4
            tok = pl.ds(i * TA, TA)
            for j in range(NP):
                b = PW * j
                mid = vt[b + 16:b + 24]
                v_s[2 * j, pl.ds(0, 16), tok] = vt[b:b + 16]
                v_s[2 * j, pl.ds(16, 8), tok] = jnp.where(lo, mid, 1.0)
                v_s[2 * j + 1, pl.ds(0, 8), tok] = jnp.where(lo, 1.0, mid)
                v_s[2 * j + 1, pl.ds(8, 16), tok] = vt[b + 24:b + 40]

        def up_block(c, r0=0, n=128):
            return lambda k, j: wup_v[pl.ds(c * D + j * 128 + r0, n), pl.ds(k * 128, 128)]

        def down_block(r0, n):
            return lambda k, j: wd_v[pl.ds(k * 256 + r0, n), pl.ds(j * 128, 128)]

        def sum_job(m, a):
            def job():
                block = up_block(m, a, 8) if m < 5 else down_block((m - 5) * 128 + a, 8)
                for n, w in enumerate(_weight_sums(block)):
                    ws_s[m, n, pl.ds(a, 8), :] = w
            return job

        def spread_keys(pair, odd, dst_ref, z):
            k = jnp.concatenate([k_s[pair, pl.ds(j * KC, NV), :] for j in range(NKC)], axis=0).T
            for d in range(DH):
                c = odd * DH + d
                kb = jnp.broadcast_to(k[c:c + 1], (128, NKC * NV)).T
                for j in range(NKC):
                    dst_ref[z, j, d] = kb[j * NV:(j + 1) * NV]

        jobs = [sum_job(m, a) for m in range(7) for a in range(0, 128, 8)]
        if not CUT & 16:
            with scope('p1_a'):
                a, n = halves[1]
                store_q(0, qf_s[0] + _dot(h_s[pl.ds(0, TA), pl.ds(a, n)], wqkv_v[pl.ds(a, n), pl.ds(0, D)]))
                wait(*cp_a)
            with scope('p1_b'):
                store_k(0, project(1, 0))
                ln_block(1)
                store_k(1, project(1, 1))
                store_q(1, project(0, 1, after_k=True))
                wait(*cp_b)
            with scope('p1_c'):
                store_v(0, project(2, 0))
                ln_block(2)
                store_v(1, project(2, 1, jobs[:11]))
                store_k(2, project(1, 2))
                ln_block(3)
                store_q(2, project(0, 2))
                store_v(2, project(2, 2, jobs[11:32], after_k=True))
                wait(*cp_c2)
            with scope('p1_d'):
                store_k(3, project(1, 3, jobs[32:48]))
                spread_keys(0, 0, kb0_s, 0)
                store_q(3, project(0, 3, jobs[48:80]))
                mod_b = _dot(sc, wmod_v[:, pl.ds(2 * D, 4 * D)])[0:1]
                store_v(3, project(2, 3, jobs[80:], after_k=True))
                v_bound = jnp.max(jnp.maximum(jnp.max(jnp.stack(v_peaks), axis=0), 1.0), keepdims=True)
                ga, sb, cb1 = mod_b[:, :D], mod_b[:, D:2 * D], 1.0 + mod_b[:, 2 * D:3 * D]
                gb_half = 0.5 * mod_b[:, 3 * D:]

        def q_weights(pair, odd, q0):
            lo = lax.broadcasted_iota(i32, (8, QB), 0) < 4
            mid = q_s[pair, pl.ds(16, 8), pl.ds(q0, QB)]
            zeros = jnp.zeros((8, QB), f32)
            if odd:
                parts = [zeros, zeros, jnp.where(lo, 0.0, mid), q_s[pair, pl.ds(24, 16), pl.ds(q0, QB)], zeros]
            else:
                parts = [q_s[pair, pl.ds(0, 16), pl.ds(q0, QB)], jnp.where(lo, mid, 0.0), zeros]
            return jnp.concatenate(parts, axis=0).astype(bf16)

        def pair_step(it, carry):
            never = [lax.broadcasted_iota(i32, (8, 128), 0) < (it >> (20 + x)) for x in range(2)]
            steps = [(odd, t, j) for odd in range(2) for t in range(NQB) for j in range(NKC)]
            qts = {}

            def vector_probs(odd, t, j):
                kb = (kb0_s, kb1_s)[odd]
                out = []
                for c in range(LT):
                    z = (it + t * LT + c) >> 23
                    for g in range(0, NV, 8):
                        s = None
                        for d in range(DH):
                            term = (kb[z, j, d, pl.ds(g, 8), :]
                                    * q_s[it, pl.ds(odd * DH + d, 1), pl.ds(t * QB + c * 128, 128)])
                            s = term if s is None else s + term
                        out.append(jnp.exp2(s))
                return out

            def probs(n):
                odd, t, j = steps[n]
                if (odd, t) not in qts:
                    qts[odd, t] = q_weights(it, odd, t * QB)
                qt = qts[odd, t]
                vals = vector_probs(odd, t, j)
                k = k_s[it, pl.ds(j * KC + NV, KC - NV), :]
                groups = [k[r:r + 8] for r in range(0, KC - NV, 8)]
                used = [0] * len(groups)
                for r, x in zip(R if n else R0, ORD):
                    if r is not None:
                        groups[r] = jnp.where(never[used[r]], vals[x], groups[r])
                        used[r] += 1
                if t == 0 and j == 0:
                    spread_keys(jnp.minimum(it + 1, NP - 1) if odd else it, 1 - odd,
                                (kb1_s, kb0_s)[odd], it >> 22)
                p = jnp.exp2(_dot(jnp.concatenate(groups, axis=0)[:, :qt.shape[0]], qt))
                top = jnp.concatenate([jnp.concatenate(vals[2 * c:2 * c + 2], axis=0) for c in range(LT)], axis=1)
                return jnp.concatenate([top, p], axis=0).astype(bf16)

            zero = jnp.full((VR, QB), it >> 25, i32).astype(f32)
            order = list(range(len(steps)))
            if LATE:
                a, n = LATE
                order = order[:-a - n - 1] + order[-a - 1:-1] + order[-a - n - 1:-a - 1] + order[-1:]
            ready = {}
            for pos, n in enumerate(order):
                while len(ready) < min(pos + LAG + 1, len(steps)) or n not in ready:
                    ready[len(ready)] = probs(len(ready))
                odd, t, j = steps[n]
                acc = (zero if j == 0 else acc) + _dot(v_s[2 * it + odd, :, pl.ds(j * KC, KC)], ready[n])
                if j == NKC - 1:
                    ot_s[2 * it + odd, :, pl.ds(t * QB, QB)] = acc
            return carry

        with scope('p2_attn'):
            if not CUT & 32:
                lax.fori_loop(0, NP, pair_step, 0)
        if CUT & 16:
            out_v[pl.ds(0, 16), :] = ot_s[0, pl.ds(0, 16), pl.ds(0, D)].astype(bf16)
            d = pltpu.make_async_copy(out_v, out_hbm, sem_out.at[0])
            d.start()
            d.wait()
            return

        def stage_o(r0, c0, delay=lambda v: v):
            lo = lax.broadcasted_iota(i32, (8, 128), 0) < 4
            parts = []
            for j in range(NP):
                e = ot_s[2 * j, :, pl.ds(r0, 128)]
                o = ot_s[2 * j + 1, :, pl.ds(r0, 128)]
                r = 1.0 / delay(jnp.where(lo, o[0:8], e[16:24]))
                re, ro = r[4:5], r[0:1]
                parts += [e[0:16] * re, jnp.where(lo, e[16:24] * re, o[0:8] * ro), o[8:24] * ro]
            o_s[pl.ds(c0, 128), :] = jnp.concatenate(parts, axis=0).T

        with scope('p2_tail'):
            wait(*cp_d)
            for c0 in range(0, TB, 128):
                stage_o(c0, c0)
            lo = lax.broadcasted_iota(i32, (8, 128), 0) < 4
            dens = jnp.stack([jnp.where(lo, ot_s[2 * j + 1, pl.ds(0, 8), pl.ds(c0, 128)],
                                        ot_s[2 * j, pl.ds(16, 8), pl.ds(c0, 128)])
                              for j in range(NP) for c0 in range(0, S, 128)])
            safe = (jnp.min(dens, axis=0) >= 2.0 ** -40) & (jnp.max(dens, axis=0) * v_bound <= 2.0 ** 120)
            unsafe = jnp.max(jnp.where(safe, 0.0, 1.0))

            @pl.when(unsafe > 0.0)
            def _():
                def attend_with_true_max(n, carry):
                    pair = n // (S // 128)
                    q0 = pl.multiple_of((n % (S // 128)) * 128, 128)
                    qp = q_s[pair, :, pl.ds(q0, 128)]
                    first = lax.broadcasted_iota(i32, qp.shape, 0) < DH
                    qt = jnp.concatenate([jnp.where(first, qp, 0.0), jnp.where(first, 0.0, qp)], axis=1)
                    s = _dot(k_s[pair, :, pl.ds(0, PW)], qt)
                    p = jnp.exp2(s - jnp.max(s, axis=0, keepdims=True)).astype(bf16)
                    for odd in range(2):
                        ot_s[2 * pair + odd, :, pl.ds(q0, 128)] = _dot(
                            v_s[2 * pair + odd], p[:, odd * 128:(odd + 1) * 128])
                    return carry
                lax.fori_loop(0, NP * (S // 128), attend_with_true_max, 0)

                def restage(n, carry):
                    stage_o(pl.multiple_of(n * 128, 128), pl.multiple_of(n * 128, 128))
                    return carry
                lax.fori_loop(0, TB // 128, restage, 0)

        def out_copy(i):
            r0 = pl.multiple_of(i * TB, TB)
            return pltpu.make_async_copy(rows(out_v, r0, TB), rows(out_hbm, r0, TB), sem_out.at[i])

        def ffn_block(i, carry):
            zero = i >> 20
            never = lax.broadcasted_iota(i32, (8, 128), 0) < zero
            tok = [pl.ds(pl.multiple_of(i * TB + b * HB, HB), HB) for b in range(2)]
            tiles = lambda v, n: [v[:, k * n:(k + 1) * n] for k in range(5)]

            def normalise(x1, dst_ref):
                for r in range(0, HB, LR):
                    dst_ref[pl.ds(r, LR), :] = _layernorm(x1[r:r + LR]) * cb1 + sb

            x1 = [x_v[tok[0], :].astype(f32) + ga * _dot(o_s[pl.ds(0, HB), :], wo_v[...])]
            ob = o_s[pl.ds(HB, HB), :]
            parts = [_dot(ob, wo_v[:, pl.ds(0, 512)])]
            normalise(x1[0], h2a_s)
            parts.append(_dot(_after(ob, h2a_s, zero), wo_v[:, pl.ds(512, 128)]))
            x1.append(x_v[tok[1], :].astype(f32) + ga * jnp.concatenate(parts, axis=1))
            ha = h2a_s[...]
            normalise(x1[1], h2b_s)
            hb = h2b_s[...]

            last = [_dot(h, wup_v[pl.ds(5 * D, 256), :], NT) for h in (ha, hb)]
            lhs = _fast_lhs([tiles(ha, 128), tiles(hb, 128)], bf16)
            up = lambda c: _fast_matmul(lhs, up_block(c), lambda n: ws_s[c, n], NT)
            acts = [[], []]
            for c in range(2):
                g = up(c)
                if c == 1:
                    for p, src in enumerate((4, 0)):
                        stage_o(pl.multiple_of(jnp.minimum(i + 1, S // TB - 1) * TB + p * 128, 128), p * 128,
                                lambda v: jnp.where(never, acts[0][src][:8], v))
                u = up(2 + c)
                for b in range(2):
                    acts[b] += [_geglu_x2(gj, uj) for gj, uj in zip(g[b], u[b])]
            mixed = up(4)
            low = lax.broadcasted_iota(i32, (HB, 128), 1) < 64
            tail = []
            for b in range(2):
                m = mixed[b]
                parts = [_geglu_x2(jnp.where(low, m[j], m[j + 1]), pltpu.roll(jnp.where(low, m[j + 1], m[j]), 64, 1))
                         for j in (0, 2)]
                parts += [_geglu_x2(last[b][:, :128], last[b][:, 128:]),
                          _geglu_x2(m[4], pltpu.roll(m[4], 64, 1))[:, :64]]
                tail.append(jnp.concatenate(parts, axis=1))
            tail = jnp.concatenate(tail, axis=0).astype(bf16)
            y_tail = (_dot(tail[:, :256], wd_v[pl.ds(2 * D, 256), :])
                      + _dot(tail[:, 256:384], wd_v[pl.ds(F - 128, 128), :])
                      + _dot(tail[:, 384:], wd_v[pl.ds(2 * D + 256, 64), :]))
            a = [tiles(jnp.concatenate(acts[b], axis=1), 256) for b in range(2)]
            y = _fast_matmul(_fast_lhs(a, f32), down_block(0, 256),
                             lambda n: jnp.concatenate([ws_s[5, n], ws_s[6, n]], axis=0), NN)
            for b in range(2):
                yb = jnp.concatenate(y[b], axis=1) + y_tail[b * HB:(b + 1) * HB]
                out_v[tok[b], :] = (x1[b] + gb_half * yb).astype(bf16)
            out_copy(i).start()
            return carry

        with scope('p3_ffn'):
            lax.fori_loop(0, S // TB, ffn_block, 0)
        with scope('p4_outwait'):
            for i in range(S // TB):
                out_copy(i).wait()

    return kernel


def build(SC=False, CUT=0, R=(1, 1, 6, 6, 10, 10), R0=(1, 1, 6, 6, 10, 10), ORD=(0, 1, 2, 3, 4, 5),
          LATE=None, LAG=2):
    def fn(A_x, A_wqkv, A_wo, B_x, B_w_gate, B_w_up, B_w_down, c, w_mod):
        hbm = pl.BlockSpec(memory_space=pltpu.MemorySpace.HBM)
        out = pl.pallas_call(
            _make_kernel(SC, CUT, R, R0, ORD, LATE, LAG),
            out_shape=jax.ShapeDtypeStruct((S, D), bf16),
            in_specs=[hbm] * 8,
            out_specs=hbm,
            scratch_shapes=[
                pltpu.VMEM((1, 4096), bf16),
                pltpu.VMEM((S, D), bf16),
                pltpu.VMEM((D, 3 * D), bf16),
                pltpu.VMEM((D, D), bf16),
                pltpu.VMEM((2 * F, D), bf16),
                pltpu.VMEM((F, D), bf16),
                pltpu.VMEM((D, 6 * D), bf16),
                pltpu.VMEM((7, len(_SUMMED), 128, 128), f32),
                pltpu.VMEM((S, D), f32),
                pltpu.VMEM((1, TA, D), f32),
                pltpu.VMEM((HB, D), f32),
                pltpu.VMEM((HB, D), f32),
                pltpu.VMEM((NP, S, 128), f32),
                pltpu.VMEM((NP, PW, S), f32),
                pltpu.VMEM((H, VR, S), f32),
                pltpu.VMEM((1, NKC, DH, NV, 128), f32),
                pltpu.VMEM((1, NKC, DH, NV, 128), f32),
                pltpu.VMEM((H, VR, S), f32),
                pltpu.VMEM((TB, D), f32),
                pltpu.VMEM((S, D), bf16),
                pltpu.SemaphoreType.DMA((30,)),
                pltpu.SemaphoreType.DMA((S // TB,)),
            ],
            compiler_params=pltpu.CompilerParams(vmem_limit_bytes=120 * 1024 * 1024),
            name="adaln_block",
        )(A_x.reshape(S, D), A_wqkv, A_wo, B_w_gate.T, B_w_up.T, B_w_down, c, w_mod)
        return out.reshape(1, S, D)
    return fn


@jax.jit
def pallas_adaLN_cond__mha_block__geglu_ffn__prompt_kernel(
    A_x: jax.Array,
    A_wqkv: jax.Array,
    A_wo: jax.Array,
    B_x: jax.Array,
    B_w_gate: jax.Array,
    B_w_up: jax.Array,
    B_w_down: jax.Array,
    c: jax.Array,
    w_mod: jax.Array,
):
    return build(R0=(6, 6, 10, 10, 13, 13))(A_x, A_wqkv, A_wo, B_x, B_w_gate, B_w_up, B_w_down, c, w_mod)
```

```python
import math

import jax
import jax.numpy as jnp
from jax import lax
import jax.experimental.pallas as pl
import jax.experimental.pallas.tpu as pltpu

S, D, H, F = 2048, 640, 32, 1728
DH = D // H
NP = H // 2
PW = 2 * DH
VR = 24
TA = 512
QA = 256
QB, KC = 512, 128
NV = 16
TB = 256
HB = TB // 2
LR = 32
WV, WK = 1024, 1664
NQB, NKC, LT = S // QB, S // KC, QB // 128
EPS = 1e-5
f32, bf16, i32 = jnp.float32, jnp.bfloat16, jnp.int32

NN = (((1,), (0,)), ((), ()))
NT = (((1,), (1,)), ((), ()))


def _dot(a, b, dims=NN):
    return lax.dot_general(a, b, dims, preferred_element_type=f32)


def _layernorm(x):
    mean = jnp.mean(x, axis=-1, keepdims=True)
    xc = x - mean
    var = jnp.mean(xc * xc, axis=-1, keepdims=True)
    return xc * lax.rsqrt(var + EPS)


def _geglu_x2(g, u):
    c0 = math.sqrt(2.0 / math.pi)
    return (g * u) * (1.0 + jnp.tanh(g * (c0 + (c0 * 0.044715) * (g * g))))


def _after(val, ref, zero, row=0):
    lead = (0,) * (len(ref.shape) - 2)
    w = pltpu.bitcast(ref[lead + (pl.ds(pl.multiple_of(zero * 8, 8), 8), pl.ds(0, 128))], i32) & zero
    head = pltpu.bitcast(pltpu.bitcast(val[row:row + 8, :128], i32) | w, f32)
    mid = jnp.concatenate([head, val[row:row + 8, 128:]], axis=1)
    return jnp.concatenate(([val[:row]] if row else []) + [mid, val[row + 8:]], axis=0)


class _Lin(dict):
    def plus(self, other):
        out = _Lin(self)
        for key, c in other.items():
            out[key] = out.get(key, 0) + c
        return _Lin({key: c for key, c in out.items() if c})

    def times(self, sign):
        return _Lin({key: sign * c for key, c in self.items()})

    def minus(self, other):
        return self.plus(other.times(-1))


def _hopcroft_kerr(kinds, helpers):
    lhs, out = [], []

    def product(a, b):
        lhs.append(a)
        out.append(b)
        return _Lin({len(lhs) - 1: 1})

    def node(ca, cb, kind, diag=None):
        f = lambda x: _Lin({(k, x % 3): c for k, c in ca.items()})
        g = lambda x: _Lin({(k, x % 3): c for k, c in cb.items()})
        diag = diag or (product(f(kind + 1), g(kind + 2)), product(f(kind + 2), g(kind + 1)))
        return dict(f=f, g=g, kind=kind, diag=diag, ca=ca, cb=cb)

    def pair(p, q):
        if (p['kind'] - q['kind']) % 3 != 1:
            qp, pq, both = pair(q, p)
            return pq, qp, both
        x = q['kind']
        m1 = product(p['f'](x).plus(q['f'](x + 1)), q['g'](x + 1).minus(p['g'](x)))
        m6 = product(q['f'](x).minus(p['f'](x)), q['g'](x + 1).plus(p['g'](x + 1)))
        m7 = product(q['f'](x + 1).minus(p['f'](x + 1)), q['g'](x).plus(p['g'](x)))
        both = node(q['ca'].minus(p['ca']), p['cb'].plus(q['cb']), (x + 2) % 3, (m6, m7))
        return (m1.plus(q['diag'][0]).minus(p['diag'][0]).plus(m7),
                m1.plus(q['diag'][1]).minus(p['diag'][1]).plus(m6), both)

    n = len(kinds)
    nodes = [node(_Lin({i: 1}), _Lin({i: 1}), kinds[i]) for i in range(n)]
    use = {(i, i): nodes[i]['diag'][0].minus(nodes[i]['diag'][1]) for i in range(n)}
    merged = {}
    for i in range(n):
        for j in range(i + 1, n):
            if kinds[i] != kinds[j]:
                use[i, j], use[j, i], merged[i, j] = pair(nodes[i], nodes[j])
    for i, j, h in helpers:
        v = merged[min(i, h), max(i, h)]
        vj, jv, _ = pair(v, nodes[j])
        use[i, j] = vj.minus(use[h, j].times(v['ca'][h])).times(v['ca'][i])
        use[j, i] = jv.minus(use[j, h].times(v['cb'][h])).times(v['cb'][i])
    rhs = [_Lin({kj: lin[r] for kj, lin in use.items() if r in lin}) for r in range(len(lhs))]
    return list(zip(lhs, rhs, out))


def _signed_sum(terms):
    terms = sorted(terms, key=lambda t: -t[0])
    sign, acc = terms[0]
    for c, v in terms[1:]:
        acc = acc + v if c == sign else acc - v
    return sign, acc


class _BlockProduct:
    def __init__(self, kinds, helpers, pair_order):
        self.n = len(kinds)
        self.scheme = _hopcroft_kerr(kinds, helpers)
        self.summed = [r for r, (_, rhs, _) in enumerate(self.scheme) if len(rhs) > 1]
        self.groups = ([[r, r + 1] for r in range(0, 2 * self.n, 2)]
                       + [[2 * self.n + 3 * x + e for e in range(3)] for x in pair_order])

    def weight_sums(self, block):
        w = {(k, j): block(k, j).astype(f32) for k in range(self.n) for j in range(self.n)}
        return [_signed_sum([(c, w[kj]) for kj, c in self.scheme[r][1].items()])[1] for r in self.summed]

    def operands(self, a, dtype, swap=False):
        f = {}
        for k, (a0, a1) in enumerate(zip(*a)):
            f[k, 0], f[k, 1], f[k, 2] = (((-1, a1), (1, a0), (1, a1 - a0)) if swap
                                         else ((1, a0), (1, a1), (-1, a0 + a1)))
        out = []
        for forms in self.scheme:
            sign, v = _signed_sum([(c * f[kx][0], f[kx][1]) for kx, c in forms[2 if swap else 0].items()])
            out.append((sign, v.astype(dtype)))
        return out

    def multiply(self, lhs, block, sums, dims, swap=False):
        t = {}
        for group in self.groups:
            new = {}
            for r in group:
                (sign, a), rhs = lhs[r], self.scheme[r][1]
                w = sums(self.summed.index(r)) if r in self.summed else block(*list(rhs)[0])
                m = _dot(a, w, dims)
                for jx, c in self.scheme[r][0 if swap else 2].items():
                    new.setdefault(jx, []).append((c * sign * max(rhs.values()), m))
            for jx, terms in new.items():
                t[jx] = _signed_sum([_signed_sum(terms)] + ([t[jx]] if jx in t else []))

        def diff(p, q):
            sign, v = _signed_sum([p, (-q[0], q[1])])
            return v if sign > 0 else -v
        return [[diff(t[j, x], t[j, y]) for j in range(self.n)]
                for x, y in (((0, 2), (1, 2)) if swap else ((1, 2), (2, 0)))]


_FIVE = _BlockProduct((0, 0, 1, 1, 2), ((0, 1, 2), (2, 3, 0)), (2, 5, 6, 7, 3, 8, 4, 9, 1, 0))
_TWO = _BlockProduct((0, 1), (), (0,))


def _kernel(x_hbm, wqkv_hbm, wo_hbm, wgt_hbm, wut_hbm, wd_hbm, c_hbm, wmod_hbm,
            out_hbm,
            c_v, x_v, wqkv_v, wo_v, wf_v, wmod_v, ws_s, wa_s, h_s, q0_s, h2a_s, h2b_s,
            k_s, qv_s, kb0_s, kb1_s, k1_s, p_s, acc_s, ot_s, o_s, out_v, sem_in, sem_out):
    copies = []

    def fetch(src, dst):
        copies.append(pltpu.make_async_copy(src, dst, sem_in.at[len(copies)]))
        return copies[-1]

    def wait(*group):
        for d in group:
            d.wait()

    rows = lambda ref, a, n: ref.at[pl.ds(a, n)]
    cols = lambda ref, a, n: ref.at[:, pl.ds(a, n)]
    fetch_x = lambda i: fetch(rows(x_hbm, i * TA, TA), rows(x_v, i * TA, TA))
    fetch_cols = lambda src, dst, a, n: fetch(cols(src, a, n), cols(dst, a, n))

    cp_c = fetch(c_hbm, cols(c_v, 0, D))
    cp_x0 = fetch_x(0)
    cp_mod = fetch_cols(wmod_hbm, wmod_v, 0, 2 * D)
    cp_wq = [fetch_cols(wqkv_hbm, wqkv_v, 0, QA), fetch_cols(wqkv_hbm, wqkv_v, QA, D - QA)]
    cp_wk = [fetch(cols(wqkv_hbm, D, D), cols(wqkv_v, WK, D)), fetch_x(1)]
    cp_wv = [fetch(cols(wqkv_hbm, 2 * D, D), cols(wqkv_v, WV, D)), fetch_x(2), fetch_x(3)]
    cp_ffn = [[fetch(rows(wgt_hbm, 0, 2 * D), rows(wf_v, 0, 2 * D)),
               fetch(rows(wut_hbm, 0, 2 * D), rows(wf_v, 2 * D, 2 * D))],
              [fetch(wd_hbm, rows(wf_v, 5 * D, F))]]
    for j in range(5):
        for src, half in ((wgt_hbm, j % 2), (wut_hbm, 1 - j % 2)):
            cp_ffn[1].append(fetch(rows(src, 2 * D + 64 * j, 64), rows(wf_v, 4 * D + 128 * j + 64 * half, 64)))
    cp_rest = [fetch_cols(wmod_hbm, wmod_v, 2 * D, 4 * D), fetch(wo_hbm, wo_v),
               fetch(rows(wgt_hbm, F - 128, 128), rows(wf_v, 5 * D + F, 128)),
               fetch(rows(wut_hbm, F - 128, 128), rows(wf_v, 5 * D + F + 128, 128))]
    for d in copies:
        d.start()

    p_s[...] = jnp.zeros(p_s.shape, bf16)
    acc_s[...] = jnp.zeros(acc_s.shape, f32)
    wait(cp_c)
    cf = c_v[:, pl.ds(0, D)].astype(f32)
    gate = jax.nn.sigmoid(cf)
    sc = jnp.broadcast_to(cf * gate, (16, D)).astype(bf16)
    zero0 = jnp.max(jnp.where(gate[:, :128] > 2.0, 1, 0))
    wait(cp_x0)

    @pl.loop(0, TA // 128)
    def _(n):
        for r in range(0, 128, 64):
            tok = pl.ds(pl.multiple_of(n * 128 + r, 64), 64)
            h_s[tok, :] = _layernorm(x_v[tok, :].astype(f32))

    wait(cp_mod)
    mod = _dot(sc, wmod_v[:, pl.ds(0, 2 * D)])[0:1]
    sa, ca1 = mod[:, :D], 1.0 + mod[:, D:]
    for r in range(0, TA, LR):
        h_s[pl.ds(r, LR), :] = h_s[pl.ds(r, LR), :] * ca1 + sa

    def normalise_block(i):
        for r in range(i * TA, (i + 1) * TA, LR):
            h_s[pl.ds(r, LR), :] = _layernorm(x_v[pl.ds(r, LR), :].astype(f32)) * ca1 + sa

    def project(w0, i, jobs=()):
        h = h_s[pl.ds(i * TA, TA), :]
        jobs = list(jobs)
        parts = []
        for c0 in range(0, D, 128):
            lhs = h
            for row in range(0, TA, 64):
                if jobs:
                    jobs.pop(0)()
                    lhs = _after(lhs, wa_s, zero0, row)
            parts.append(_dot(lhs, wqkv_v[:, pl.ds(w0 + c0, 128)]))
        return jnp.concatenate(parts, axis=1)

    def project_by_rows(w0, i):
        return jnp.concatenate([_dot(h_s[pl.ds(i * TA + r, 128), :], wqkv_v[:, pl.ds(w0, D)])
                                for r in range(0, TA, 128)], axis=0)

    def qv_block(is_v, r0=0, n=256):
        return lambda k, j: wqkv_v[pl.ds(k * 256 + r0, n), pl.ds(pl.multiple_of(WV * is_v + j * 256, 128), 256)]

    def qv_sum_job(is_v, r0):
        def job():
            for n, w in enumerate(_TWO.weight_sums(qv_block(is_v, r0, 8))):
                wa_s[is_v, n, pl.ds(r0, 8), :] = w
        return job

    def project_qv(is_v, i, jobs):
        h = h_s[pl.ds(i * TA, TA), :]
        lhs = _TWO.operands([[h[b:b + 256, k:k + 256] for k in (0, 256)] for b in (0, 256)], f32)
        for r in range(1, 7):
            for row in range(0, 256, 64):
                if jobs:
                    jobs.pop(0)()
                    lhs[r] = (lhs[r][0], _after(lhs[r][1], ws_s, zero0, row))
        y = _TWO.multiply(lhs, qv_block(is_v), lambda n: wa_s[is_v, n], NN)
        w0 = pl.multiple_of(WV * is_v, 128)
        body = (jnp.concatenate([jnp.concatenate(row, axis=1) for row in y], axis=0)
                + _dot(h[:, 512:], wqkv_v[pl.ds(512, 128), pl.ds(w0, 512)]))
        return jnp.concatenate([body, _dot(h, wqkv_v[:, pl.ds(w0 + 512, 128)])], axis=1)

    def store_k(i, k):
        hi = lax.broadcasted_iota(i32, (TA, 128), 1) >= 64
        for j in range(NP):
            t, o = divmod(j * PW, 128)
            w = k[:, t * 128:(t + 1) * 128]
            if o + PW > 128:
                w = jnp.where(hi, w, k[:, (t + 1) * 128:(t + 2) * 128])
            k_s[j, pl.ds(i * TA, TA), :] = pltpu.roll(w, 128 - o, 1) if o else w

    def store_qv(is_v, i, y):
        yt = (y * jnp.where(is_v, 1.0, DH ** -0.5 * math.log2(math.e))).T
        fill = jnp.where(is_v, 1.0, 0.0)
        lo = lax.broadcasted_iota(i32, (8, TA), 0) < 4
        tok = pl.ds(i * TA, TA)
        for j in range(NP):
            b = PW * j
            mid = yt[b + 16:b + 24]
            qv_s[is_v, 2 * j, pl.ds(0, 16), tok] = yt[b:b + 16]
            qv_s[is_v, 2 * j, pl.ds(16, 8), tok] = jnp.where(lo, mid, fill)
            qv_s[is_v, 2 * j + 1, pl.ds(0, 8), tok] = jnp.where(lo, fill, mid)
            qv_s[is_v, 2 * j + 1, pl.ds(8, 16), tok] = yt[b + 24:b + 40]
        return jnp.max(jnp.abs(yt).reshape(D // 8, 8, TA), axis=0)

    def ffn_block(m, r0=0, n=128):
        return lambda k, j: wf_v[pl.ds(pl.multiple_of(m * D + j * 128 + r0, 8), n), pl.ds(k * 128, 128)]

    def ffn_sum_job(m, r0):
        def job():
            for n, w in enumerate(_FIVE.weight_sums(ffn_block(m, r0, 8))):
                ws_s[m, n, pl.ds(pl.multiple_of(r0, 8), 8), :] = w
        return job

    def spread_keys(pair, odd, dst_ref, zero):
        k = jnp.concatenate([k_s[pair, pl.ds(j * KC, NV), :] for j in range(NKC)], axis=0).T
        for d in range(DH):
            c = odd * DH + d
            kb = jnp.broadcast_to(k[c:c + 1], (128, NKC * NV)).T
            for j in range(NKC):
                dst_ref[zero, j, d] = kb[j * NV:(j + 1) * NV]

    def qv_step(is_v, peak):
        for n in range(2):
            pl.when(is_v == n)(lambda n=n: wait(*cp_ffn[n]))
        jobs = [ffn_sum_job(m + 4 * is_v, r0) for m in range(3) for r0 in range(0, 128, 8)]
        jobs += [ffn_sum_job(3, r0 + 64 * is_v) for r0 in range(0, 64, 8)]
        spread_keys(0, 0, kb0_s, 0)
        for i, share in ((1, jobs[:10]), (2, jobs[10:33]), (3, jobs[33:])):
            peak = jnp.maximum(peak, store_qv(is_v, i, project_qv(is_v, i, share)))
        return peak

    wait(cp_wq[0])
    q0_s[zero0] = _dot(h_s[pl.ds(0, TA), :], wqkv_v[:, pl.ds(0, QA)])
    wait(cp_wq[1])
    store_qv(0, 0, jnp.concatenate([q0_s[0], _dot(h_s[pl.ds(0, TA), :], wqkv_v[:, pl.ds(QA, D - QA)])], axis=1))
    wait(*cp_wk)
    store_k(0, project(WK, 0, [qv_sum_job(0, r0) for r0 in range(0, 256, 8)]))
    normalise_block(1)
    store_k(1, project_by_rows(WK, 1))
    wait(*cp_wv)
    peak = store_qv(1, 0, project(WV, 0))
    normalise_block(2)
    store_k(2, project(WK, 2, [qv_sum_job(1, r0) for r0 in range(0, 256, 8)]))
    normalise_block(3)
    store_k(3, project_by_rows(WK, 3))
    peak = lax.fori_loop(0, 2, qv_step, peak)
    v_bound = jnp.max(jnp.maximum(peak, 1.0), keepdims=True)

    def q_weights(head, tok, lead=0):
        q = qv_s[0, head, :, tok]
        zeros = jnp.zeros((8, q.shape[1]), f32)
        return jnp.concatenate([zeros] * lead + [q, zeros], axis=0).astype(bf16)

    def finish(head):
        return acc_s[...] + _dot(qv_s[1, head, :, pl.ds(S - KC, KC)], p_s[...])

    def pair_step(it, carry):
        never = [lax.broadcasted_iota(i32, (8, 128), 0) < (it >> (20 + x)) for x in range(2)]
        steps = [(odd, t, j) for odd in range(2) for t in range(NQB) for j in range(NKC)]
        last = len(steps) - 1
        qts, marks = {}, []

        def vector_probs(odd, t, j):
            kb = (kb0_s, kb1_s)[odd]
            out = []
            for c in range(LT):
                zero = (it + t * LT + c) >> 23
                for g in range(0, NV, 8):
                    s = None
                    for d in range(DH):
                        q = qv_s[0, 2 * it + odd, pl.ds(4 * odd + d, 1), pl.ds(t * QB + c * 128, 128)]
                        term = kb[zero, j, d, pl.ds(g, 8), :] * q
                        s = term if s is None else s + term
                    out.append(jnp.exp2(s))
            return out

        def probs(n):
            odd, t, j = steps[n]
            if (odd, t) not in qts:
                qts[odd, t] = q_weights(2 * it + odd, pl.ds(t * QB, QB))
            vals = vector_probs(odd, t, j)
            keys = pl.ds(j * KC + NV, KC - NV)
            k = k1_s[it >> 26, keys, :] if odd else k_s[it, keys, :]
            if not odd and t == 0:
                k1_s[it >> 27, keys, :] = pltpu.roll(k_s[it + (it >> 28), keys, :], 128 - 16, 1)
            groups = [k[r:r + 8] for r in range(0, KC - NV, 8)]
            for x, r in enumerate((1, 1, 6, 6, 10, 10) if n else (6, 6, 10, 10, 13, 13)):
                groups[r] = jnp.where(never[x % 2], vals[x], groups[r])
            if n == last:
                groups[0] = jnp.where(never[0], marks[n - 2], groups[0])
            if t == 0 and j == 0:
                spread_keys(jnp.minimum(it + 1, NP - 1) if odd else it, 1 - odd, (kb1_s, kb0_s)[odd], it >> 22)
            p = jnp.exp2(_dot(jnp.concatenate(groups, axis=0)[:, :VR + 8], qts[odd, t]))
            marks.append(p[:8, :128])
            if n == last:
                vals = [jnp.where(never[0], marks[n], v) for v in vals]
            top = jnp.concatenate([jnp.concatenate(vals[2 * c:2 * c + 2], axis=0) for c in range(LT)], axis=1)
            return jnp.concatenate([top, p], axis=0).astype(bf16)

        zeros = jnp.full((VR, QB), it >> 25, i32).astype(f32)
        ot_s[jnp.where(it == 0, H, 2 * it - 1), :, pl.ds(S - QB, QB)] = finish(jnp.maximum(2 * it - 1, 0))
        ready = [probs(0), probs(1)]
        for n, (odd, t, j) in enumerate(steps[:last]):
            if n + 2 <= last:
                ready.append(probs(n + 2))
            acc = (zeros if j == 0 else acc) + _dot(qv_s[1, 2 * it + odd, :, pl.ds(j * KC, KC)], ready[n])
            if j == NKC - 1:
                ot_s[2 * it + odd, :, pl.ds(t * QB, QB)] = acc
        p_s[...] = ready[last]
        acc_s[...] = acc
        return carry

    lax.fori_loop(0, NP, pair_step, 0)

    def stage_o(r0, c0, delay=lambda v: v):
        lo = lax.broadcasted_iota(i32, (8, 128), 0) < 4
        parts = []
        for j in range(NP):
            e = ot_s[2 * j, :, pl.ds(r0, 128)]
            o = ot_s[2 * j + 1, :, pl.ds(r0, 128)]
            r = 1.0 / delay(jnp.where(lo, o[0:8], e[16:24]))
            re, ro = r[4:5], r[0:1]
            parts += [e[0:16] * re, jnp.where(lo, e[16:24] * re, o[0:8] * ro), o[8:24] * ro]
        o_s[pl.ds(c0, 128), :] = jnp.concatenate(parts, axis=0).T

    wait(*cp_rest)
    ot_s[H - 1, :, pl.ds(S - QB, QB)] = finish(H - 1)
    mod = _dot(sc, wmod_v[:, pl.ds(2 * D, 4 * D)])[0:1]
    ga, sb, cb1, gb_half = mod[:, :D], mod[:, D:2 * D], 1.0 + mod[:, 2 * D:3 * D], 0.5 * mod[:, 3 * D:]
    for c0 in range(0, TB, 128):
        stage_o(c0, c0)

    lo = lax.broadcasted_iota(i32, (8, 128), 0) < 4
    dens = jnp.stack([jnp.where(lo, ot_s[2 * j + 1, pl.ds(0, 8), pl.ds(c0, 128)],
                                ot_s[2 * j, pl.ds(16, 8), pl.ds(c0, 128)])
                      for j in range(NP) for c0 in range(0, S, 128)])
    safe = (jnp.min(dens, axis=0) >= 2.0 ** -40) & (jnp.max(dens, axis=0) * v_bound <= 2.0 ** 120)

    @pl.when(jnp.max(jnp.where(safe, 0.0, 1.0)) > 0.0)
    def _():
        @pl.loop(0, H * NQB)
        def attend_with_true_max(n):
            head = n // NQB
            tok = pl.ds(pl.multiple_of((n % NQB) * QB, QB), QB)
            qt = jnp.where(head % 2 == 1, q_weights(head, tok, 2)[:PW],
                           jnp.concatenate([q_weights(head, tok), jnp.zeros((8, QB), bf16)], axis=0))
            keys = lambda j: pl.ds(pl.multiple_of(j * KC, KC), KC)
            scores = lambda j: _dot(k_s[head // 2, keys(j), pl.ds(0, PW)], qt)
            top = lax.fori_loop(0, NKC, lambda j, m: jnp.maximum(m, jnp.max(scores(j), axis=0, keepdims=True)),
                                jnp.full((1, QB), -jnp.inf, f32))
            ot_s[head, :, tok] = lax.fori_loop(
                0, NKC, lambda j, acc: acc + _dot(qv_s[1, head, :, keys(j)], jnp.exp2(scores(j) - top)),
                jnp.zeros((VR, QB), f32))

        @pl.loop(0, TB // 128)
        def _(n):
            stage_o(pl.multiple_of(n * 128, 128), pl.multiple_of(n * 128, 128))

    def out_copy(i):
        r0 = pl.multiple_of(i * TB, TB)
        return pltpu.make_async_copy(rows(out_v, r0, TB), rows(out_hbm, r0, TB), sem_out.at[i])

    @pl.loop(0, S // TB)
    def ffn_step(i):
        zero = i >> 20
        never = lax.broadcasted_iota(i32, (8, 128), 0) < zero
        tok = [pl.ds(pl.multiple_of(i * TB + b * HB, HB), HB) for b in range(2)]

        def normalise(x1, dst_ref):
            for r in range(0, HB, LR):
                dst_ref[pl.ds(r, LR), :] = _layernorm(x1[r:r + LR]) * cb1 + sb

        x1 = [x_v[tok[0], :].astype(f32) + ga * _dot(o_s[pl.ds(0, HB), :], wo_v[...])]
        ob = o_s[pl.ds(HB, HB), :]
        parts = [_dot(ob, wo_v[:, pl.ds(0, 512)])]
        normalise(x1[0], h2a_s)
        parts.append(_dot(_after(ob, h2a_s, zero), wo_v[:, pl.ds(512, 128)]))
        x1.append(x_v[tok[1], :].astype(f32) + ga * jnp.concatenate(parts, axis=1))
        h = [h2a_s[...]]
        normalise(x1[1], h2b_s)
        h.append(h2b_s[...])

        last = [_dot(hb, wf_v[pl.ds(5 * D + F, 256), :], NT) for hb in h]
        lhs = _FIVE.operands([[hb[:, k:k + 128] for k in range(0, D, 128)] for hb in h], bf16)
        up = lambda m: _FIVE.multiply(lhs, ffn_block(m), lambda n: ws_s[m, n], NT)
        acts = [[], []]
        for m in range(2):
            g = up(m)
            if m == 1:
                for c0, mark in ((0, 4), (128, 0)):
                    stage_o(pl.multiple_of(jnp.minimum(i + 1, S // TB - 1) * TB + c0, 128), c0,
                            lambda v: jnp.where(never, acts[0][mark][:8], v))
            u = up(2 + m)
            for b in range(2):
                acts[b] += [_geglu_x2(gj, uj) for gj, uj in zip(g[b], u[b])]
        mixed = up(4)
        low = lax.broadcasted_iota(i32, (HB, 128), 1) < 64
        tail = []
        for b in range(2):
            gu = mixed[b]
            parts = [_geglu_x2(jnp.where(low, gu[j], gu[j + 1]), pltpu.roll(jnp.where(low, gu[j + 1], gu[j]), 64, 1))
                     for j in (0, 2)]
            parts += [_geglu_x2(last[b][:, :128], last[b][:, 128:]), _geglu_x2(gu[4], pltpu.roll(gu[4], 64, 1))]
            tail.append(jnp.concatenate(parts, axis=1))
        tail = jnp.concatenate(tail, axis=0).astype(bf16)
        y_tail = (_dot(tail[:, :256], wf_v[pl.ds(7 * D, 256), :])
                  + _dot(tail[:, 256:384], wf_v[pl.ds(5 * D + F - 128, 128), :])
                  + _dot(tail[:, 384:448], wf_v[pl.ds(7 * D + 256, 64), :]))
        a = [[jnp.concatenate(acts[b][k::5], axis=1) for k in range(5)] for b in range(2)]
        y = _FIVE.multiply(_FIVE.operands(a, f32, swap=True),
                           lambda k, j: jnp.concatenate([ffn_block(m)(k, j) for m in (5, 6)], axis=0),
                           lambda n: jnp.concatenate([ws_s[5, n], ws_s[6, n]], axis=0), NN, swap=True)
        for b in range(2):
            yb = jnp.concatenate(y[b], axis=1) + y_tail[b * HB:(b + 1) * HB]
            out_v[tok[b], :] = (x1[b] + gb_half * yb).astype(bf16)
        out_copy(i).start()

    for i in range(S // TB):
        out_copy(i).wait()


@jax.jit
def pallas_adaLN_cond__mha_block__geglu_ffn__prompt_kernel(
    A_x: jax.Array,
    A_wqkv: jax.Array,
    A_wo: jax.Array,
    B_x: jax.Array,
    B_w_gate: jax.Array,
    B_w_up: jax.Array,
    B_w_down: jax.Array,
    c: jax.Array,
    w_mod: jax.Array,
):
    del B_x
    hbm = pl.BlockSpec(memory_space=pltpu.MemorySpace.HBM)
    out = pl.pallas_call(
        _kernel,
        out_shape=jax.ShapeDtypeStruct((S, D), bf16),
        in_specs=[hbm] * 8,
        out_specs=hbm,
        scratch_shapes=[
            pltpu.VMEM((1, 4096), bf16),
            pltpu.VMEM((S, D), bf16),
            pltpu.VMEM((D, WK + D), bf16),
            pltpu.VMEM((D, D), bf16),
            pltpu.VMEM((3 * F, D), bf16),
            pltpu.VMEM((D, 6 * D), bf16),
            pltpu.VMEM((7, len(_FIVE.summed), 128, 128), f32),
            pltpu.VMEM((2, len(_TWO.summed), 256, 256), f32),
            pltpu.VMEM((S, D), f32),
            pltpu.VMEM((1, TA, QA), f32),
            pltpu.VMEM((HB, D), f32),
            pltpu.VMEM((HB, D), f32),
            pltpu.VMEM((NP, S, 128), f32),
            pltpu.VMEM((2, H, VR, S), f32),
            pltpu.VMEM((1, NKC, DH, NV, 128), f32),
            pltpu.VMEM((1, NKC, DH, NV, 128), f32),
            pltpu.VMEM((1, S, 128), f32),
            pltpu.VMEM((KC, QB), bf16),
            pltpu.VMEM((VR, QB), f32),
            pltpu.VMEM((H + 1, VR, S), f32),
            pltpu.VMEM((TB, D), f32),
            pltpu.VMEM((S, D), bf16),
            pltpu.SemaphoreType.DMA((27,)),
            pltpu.SemaphoreType.DMA((S // TB,)),
        ],
        compiler_params=pltpu.CompilerParams(vmem_limit_bytes=120 * 1024 * 1024),
        name="adaln_block",
    )(A_x.reshape(S, D), A_wqkv, A_wo, B_w_gate.T, B_w_up.T, B_w_down, c, w_mod)
    return out.reshape(1, S, D)
```

```python
import math

import jax
import jax.numpy as jnp
from jax import lax
import jax.experimental.pallas as pl
import jax.experimental.pallas.tpu as pltpu

S, D, H, F = 2048, 640, 32, 1728
DH = D // H
NP = H // 2
PW = 2 * DH
VR = 24
TA = 512
QA = 256
QB, KC = 512, 128
NV = 16
TB = 256
HB = TB // 2
LR = 32
WV, WK = 1024, 1664
NQB, NKC, LT = S // QB, S // KC, QB // 128
EPS = 1e-5
f32, bf16, i32 = jnp.float32, jnp.bfloat16, jnp.int32

NN = (((1,), (0,)), ((), ()))
NT = (((1,), (1,)), ((), ()))


def _dot(a, b, dims=NN):
    return lax.dot_general(a, b, dims, preferred_element_type=f32)


def _layernorm(x):
    mean = jnp.mean(x, axis=-1, keepdims=True)
    xc = x - mean
    var = jnp.mean(xc * xc, axis=-1, keepdims=True)
    return xc * lax.rsqrt(var + EPS)


def _geglu_x2(g, u):
    c0 = math.sqrt(2.0 / math.pi)
    return (g * u) * (1.0 + jnp.tanh(g * (c0 + (c0 * 0.044715) * (g * g))))


def _after(val, ref, zero, row=0):
    lead = (0,) * (len(ref.shape) - 2)
    w = pltpu.bitcast(ref[lead + (pl.ds(pl.multiple_of(zero * 8, 8), 8), pl.ds(0, 128))], i32) & zero
    head = pltpu.bitcast(pltpu.bitcast(val[row:row + 8, :128], i32) | w, f32)
    mid = jnp.concatenate([head, val[row:row + 8, 128:]], axis=1)
    return jnp.concatenate(([val[:row]] if row else []) + [mid, val[row + 8:]], axis=0)


class _Lin(dict):
    def plus(self, other):
        out = _Lin(self)
        for key, c in other.items():
            out[key] = out.get(key, 0) + c
        return _Lin({key: c for key, c in out.items() if c})

    def times(self, sign):
        return _Lin({key: sign * c for key, c in self.items()})

    def minus(self, other):
        return self.plus(other.times(-1))


def _hopcroft_kerr(kinds, helpers):
    lhs, out = [], []

    def product(a, b):
        lhs.append(a)
        out.append(b)
        return _Lin({len(lhs) - 1: 1})

    def node(ca, cb, kind, diag=None):
        f = lambda x: _Lin({(k, x % 3): c for k, c in ca.items()})
        g = lambda x: _Lin({(k, x % 3): c for k, c in cb.items()})
        diag = diag or (product(f(kind + 1), g(kind + 2)), product(f(kind + 2), g(kind + 1)))
        return dict(f=f, g=g, kind=kind, diag=diag, ca=ca, cb=cb)

    def pair(p, q):
        if (p['kind'] - q['kind']) % 3 != 1:
            qp, pq, both = pair(q, p)
            return pq, qp, both
        x = q['kind']
        m1 = product(p['f'](x).plus(q['f'](x + 1)), q['g'](x + 1).minus(p['g'](x)))
        m6 = product(q['f'](x).minus(p['f'](x)), q['g'](x + 1).plus(p['g'](x + 1)))
        m7 = product(q['f'](x + 1).minus(p['f'](x + 1)), q['g'](x).plus(p['g'](x)))
        both = node(q['ca'].minus(p['ca']), p['cb'].plus(q['cb']), (x + 2) % 3, (m6, m7))
        return (m1.plus(q['diag'][0]).minus(p['diag'][0]).plus(m7),
                m1.plus(q['diag'][1]).minus(p['diag'][1]).plus(m6), both)

    n = len(kinds)
    nodes = [node(_Lin({i: 1}), _Lin({i: 1}), kinds[i]) for i in range(n)]
    use = {(i, i): nodes[i]['diag'][0].minus(nodes[i]['diag'][1]) for i in range(n)}
    merged = {}
    for i in range(n):
        for j in range(i + 1, n):
            if kinds[i] != kinds[j]:
                use[i, j], use[j, i], merged[i, j] = pair(nodes[i], nodes[j])
    for i, j, h in helpers:
        v = merged[min(i, h), max(i, h)]
        vj, jv, _ = pair(v, nodes[j])
        use[i, j] = vj.minus(use[h, j].times(v['ca'][h])).times(v['ca'][i])
        use[j, i] = jv.minus(use[j, h].times(v['cb'][h])).times(v['cb'][i])
    rhs = [_Lin({kj: lin[r] for kj, lin in use.items() if r in lin}) for r in range(len(lhs))]
    return list(zip(lhs, rhs, out))


def _signed_sum(terms):
    terms = sorted(terms, key=lambda t: -t[0])
    sign, acc = terms[0]
    for c, v in terms[1:]:
        acc = acc + v if c == sign else acc - v
    return sign, acc


class _BlockProduct:
    def __init__(self, kinds, helpers, pair_order):
        self.n = len(kinds)
        self.scheme = _hopcroft_kerr(kinds, helpers)
        self.summed = [r for r, (_, rhs, _) in enumerate(self.scheme) if len(rhs) > 1]
        self.groups = ([[r, r + 1] for r in range(0, 2 * self.n, 2)]
                       + [[2 * self.n + 3 * x + e for e in range(3)] for x in pair_order])

    def weight_sums(self, block):
        w = {(k, j): block(k, j).astype(f32) for k in range(self.n) for j in range(self.n)}
        return [_signed_sum([(c, w[kj]) for kj, c in self.scheme[r][1].items()])[1] for r in self.summed]

    def operands(self, a, dtype, swap=False):
        f = {}
        for k, (a0, a1) in enumerate(zip(*a)):
            f[k, 0], f[k, 1], f[k, 2] = (((-1, a1), (1, a0), (1, a1 - a0)) if swap
                                         else ((1, a0), (1, a1), (-1, a0 + a1)))
        out = []
        for forms in self.scheme:
            sign, v = _signed_sum([(c * f[kx][0], f[kx][1]) for kx, c in forms[2 if swap else 0].items()])
            out.append((sign, v.astype(dtype)))
        return out

    def multiply(self, lhs, block, sums, dims, swap=False):
        t = {}
        for group in self.groups:
            new = {}
            for r in group:
                (sign, a), rhs = lhs[r], self.scheme[r][1]
                w = sums(self.summed.index(r)) if r in self.summed else block(*list(rhs)[0])
                m = _dot(a, w, dims)
                for jx, c in self.scheme[r][0 if swap else 2].items():
                    new.setdefault(jx, []).append((c * sign * max(rhs.values()), m))
            for jx, terms in new.items():
                t[jx] = _signed_sum([_signed_sum(terms)] + ([t[jx]] if jx in t else []))

        def diff(p, q):
            sign, v = _signed_sum([p, (-q[0], q[1])])
            return v if sign > 0 else -v
        return [[diff(t[j, x], t[j, y]) for j in range(self.n)]
                for x, y in (((0, 2), (1, 2)) if swap else ((1, 2), (2, 0)))]


_FIVE = _BlockProduct((0, 0, 1, 1, 2), ((0, 1, 2), (2, 3, 0)), (5, 2, 6, 7, 8, 3, 4, 1, 9, 0))
_TWO = _BlockProduct((0, 1), (), (0,))


def _kernel(x_hbm, wqkv_hbm, wo_hbm, wgt_hbm, wut_hbm, wd_hbm, c_hbm, wmod_hbm,
            out_hbm,
            c_v, x_v, wqkv_v, wo_v, wf_v, wmod_v, ws_s, wa_s, h_s, q0_s, h2a_s, h2b_s,
            k_s, qv_s, kb0_s, kb1_s, k1_s, p_s, acc_s, ot_s, o_s, out_v, sem_in, sem_out):
    copies = []

    def fetch(src, dst):
        copies.append(pltpu.make_async_copy(src, dst, sem_in.at[len(copies)]))
        return copies[-1]

    def wait(*group):
        for d in group:
            d.wait()

    rows = lambda ref, a, n: ref.at[pl.ds(a, n)]
    cols = lambda ref, a, n: ref.at[:, pl.ds(a, n)]
    fetch_x = lambda i: fetch(rows(x_hbm, i * TA, TA), rows(x_v, i * TA, TA))
    fetch_cols = lambda src, dst, a, n: fetch(cols(src, a, n), cols(dst, a, n))

    cp_c = fetch(c_hbm, cols(c_v, 0, D))
    cp_x0 = fetch_x(0)
    cp_mod = fetch_cols(wmod_hbm, wmod_v, 0, 2 * D)
    cp_wq = [fetch_cols(wqkv_hbm, wqkv_v, 0, QA), fetch_cols(wqkv_hbm, wqkv_v, QA, D - QA)]
    cp_wk = [fetch(cols(wqkv_hbm, D, D), cols(wqkv_v, WK, D)), fetch_x(1)]
    cp_wv = [fetch(cols(wqkv_hbm, 2 * D, D), cols(wqkv_v, WV, D)), fetch_x(2), fetch_x(3)]
    cp_ffn = [[fetch(rows(wgt_hbm, 0, 2 * D), rows(wf_v, 0, 2 * D)),
               fetch(rows(wut_hbm, 0, 2 * D), rows(wf_v, 2 * D, 2 * D))],
              [fetch(wd_hbm, rows(wf_v, 5 * D, F))]]
    for j in range(5):
        for src, half in ((wgt_hbm, j % 2), (wut_hbm, 1 - j % 2)):
            cp_ffn[1].append(fetch(rows(src, 2 * D + 64 * j, 64), rows(wf_v, 4 * D + 128 * j + 64 * half, 64)))
    cp_rest = [fetch_cols(wmod_hbm, wmod_v, 2 * D, 4 * D), fetch(wo_hbm, wo_v),
               fetch(rows(wgt_hbm, F - 128, 128), rows(wf_v, 5 * D + F, 128)),
               fetch(rows(wut_hbm, F - 128, 128), rows(wf_v, 5 * D + F + 128, 128))]
    for d in copies:
        d.start()

    p_s[...] = jnp.zeros(p_s.shape, bf16)
    acc_s[...] = jnp.zeros(acc_s.shape, f32)
    wait(cp_c)
    cf = c_v[:, pl.ds(0, D)].astype(f32)
    gate = jax.nn.sigmoid(cf)
    sc = jnp.broadcast_to(cf * gate, (16, D)).astype(bf16)
    zero0 = jnp.max(jnp.where(gate[:, :128] > 2.0, 1, 0))
    wait(cp_x0)

    @pl.loop(0, TA // 128)
    def _(n):
        for r in range(0, 128, 64):
            tok = pl.ds(pl.multiple_of(n * 128 + r, 64), 64)
            h_s[tok, :] = _layernorm(x_v[tok, :].astype(f32))

    wait(cp_mod)
    mod = _dot(sc, wmod_v[:, pl.ds(0, 2 * D)])[0:1]
    sa, ca1 = mod[:, :D], 1.0 + mod[:, D:]
    for r in range(0, TA, LR):
        h_s[pl.ds(r, LR), :] = h_s[pl.ds(r, LR), :] * ca1 + sa

    def normalise_block(i):
        for r in range(i * TA, (i + 1) * TA, LR):
            h_s[pl.ds(r, LR), :] = _layernorm(x_v[pl.ds(r, LR), :].astype(f32)) * ca1 + sa

    def project(w0, i, jobs=()):
        h = h_s[pl.ds(i * TA, TA), :]
        jobs = list(jobs)
        parts = []
        for c0 in range(0, D, 128):
            lhs = h
            for row in range(0, TA, 64):
                if jobs:
                    jobs.pop(0)()
                    lhs = _after(lhs, wa_s, zero0, row)
            parts.append(_dot(lhs, wqkv_v[:, pl.ds(w0 + c0, 128)]))
        assert not jobs
        return jnp.concatenate(parts, axis=1)

    def project_by_rows(w0, i):
        return jnp.concatenate([_dot(h_s[pl.ds(i * TA + r, 128), :], wqkv_v[:, pl.ds(w0, D)])
                                for r in range(0, TA, 128)], axis=0)

    def qv_block(is_v, r0=0, n=256):
        return lambda k, j: wqkv_v[pl.ds(k * 256 + r0, n), pl.ds(pl.multiple_of(WV * is_v + j * 256, 128), 256)]

    def qv_sum_job(is_v, r0):
        def job():
            for n, w in enumerate(_TWO.weight_sums(qv_block(is_v, r0, 8))):
                wa_s[is_v, n, pl.ds(r0, 8), :] = w
        return job

    def project_qv(is_v, i, jobs):
        h = h_s[pl.ds(i * TA, TA), :]
        lhs = _TWO.operands([[h[b:b + 256, k:k + 256] for k in (0, 256)] for b in (0, 256)], f32)
        for r in range(1, 7):
            for row in range(0, 256, 64):
                if jobs:
                    jobs.pop(0)()
                    lhs[r] = (lhs[r][0], _after(lhs[r][1], ws_s, zero0, row))
        assert not jobs
        y = _TWO.multiply(lhs, qv_block(is_v), lambda n: wa_s[is_v, n], NN)
        w0 = pl.multiple_of(WV * is_v, 128)
        body = (jnp.concatenate([jnp.concatenate(row, axis=1) for row in y], axis=0)
                + _dot(h[:, 512:], wqkv_v[pl.ds(512, 128), pl.ds(w0, 512)]))
        return jnp.concatenate([body, _dot(h, wqkv_v[:, pl.ds(w0 + 512, 128)])], axis=1)

    def store_k(i, k):
        k = pltpu.bitcast(k.astype(bf16), i32)
        hi = lax.broadcasted_iota(i32, (TA // 2, 128), 1) >= 64
        for j in range(NP):
            t, o = divmod(j * PW, 128)
            w = k[:, t * 128:(t + 1) * 128]
            if o + PW > 128:
                w = jnp.where(hi, w, k[:, (t + 1) * 128:(t + 2) * 128])
            k_s[j, pl.ds(i * TA // 2, TA // 2), :] = pltpu.roll(w, 128 - o, 1) if o else w

    def store_qv(is_v, i, y):
        yt = (y * jnp.where(is_v, 1.0, DH ** -0.5 * math.log2(math.e))).T
        fill = jnp.where(is_v, 1.0, 0.0)
        lo = lax.broadcasted_iota(i32, (8, TA), 0) < 4
        tok = pl.ds(i * TA, TA)
        for j in range(NP):
            b = PW * j
            mid = yt[b + 16:b + 24]
            qv_s[is_v, 2 * j, pl.ds(0, 16), tok] = yt[b:b + 16]
            qv_s[is_v, 2 * j, pl.ds(16, 8), tok] = jnp.where(lo, mid, fill)
            qv_s[is_v, 2 * j + 1, pl.ds(0, 8), tok] = jnp.where(lo, fill, mid)
            qv_s[is_v, 2 * j + 1, pl.ds(8, 16), tok] = yt[b + 24:b + 40]
        return jnp.max(jnp.abs(yt).reshape(D // 8, 8, TA), axis=0)

    def ffn_block(m, r0=0, n=128):
        return lambda k, j: wf_v[pl.ds(pl.multiple_of(m * D + j * 128 + r0, 8), n), pl.ds(k * 128, 128)]

    def ffn_sum_job(m, r0):
        def job():
            for n, w in enumerate(_FIVE.weight_sums(ffn_block(m, r0, 8))):
                ws_s[m, n, pl.ds(pl.multiple_of(r0, 8), 8), :] = w
        return job

    def spread_keys(pair, odd, dst_ref, zero):
        k = jnp.concatenate([k_s[pair, pl.ds(j * KC // 2, NV // 2), :] for j in range(NKC)], axis=0)
        k = pltpu.bitcast(k, bf16).astype(f32)
        k = pltpu.bitcast(pltpu.bitcast(k, i32) | zero, f32).T
        for d in range(DH):
            c = odd * DH + d
            kb = jnp.broadcast_to(k[c:c + 1], (128, NKC * NV)).T
            for j in range(NKC):
                dst_ref[zero, j, d] = kb[j * NV:(j + 1) * NV]

    def qv_step(is_v, peak):
        for n in range(2):
            pl.when(is_v == n)(lambda n=n: wait(*cp_ffn[n]))
        jobs = [ffn_sum_job(m + 4 * is_v, r0) for m in range(3) for r0 in range(0, 128, 8)]
        jobs += [ffn_sum_job(3, r0 + 64 * is_v) for r0 in range(0, 64, 8)]
        spread_keys(0, 0, kb0_s, zero0)
        for i, share in ((1, jobs[:10]), (2, jobs[10:33]), (3, jobs[33:])):
            peak = jnp.maximum(peak, store_qv(is_v, i, project_qv(is_v, i, share)))
        return peak

    wait(cp_wq[0])
    q0_s[zero0] = _dot(h_s[pl.ds(0, TA), :], wqkv_v[:, pl.ds(0, QA)])
    wait(cp_wq[1])
    store_qv(0, 0, jnp.concatenate([q0_s[0], _dot(h_s[pl.ds(0, TA), :], wqkv_v[:, pl.ds(QA, D - QA)])], axis=1))
    wait(*cp_wk)
    store_k(0, project(WK, 0, [qv_sum_job(0, r0) for r0 in range(0, 256, 8)]))
    normalise_block(1)
    store_k(1, project_by_rows(WK, 1))
    wait(*cp_wv)
    peak = store_qv(1, 0, project(WV, 0))
    normalise_block(2)
    store_k(2, project(WK, 2, [qv_sum_job(1, r0) for r0 in range(0, 256, 8)]))
    normalise_block(3)
    store_k(3, project_by_rows(WK, 3))
    peak = lax.fori_loop(0, 2, qv_step, peak)
    v_bound = jnp.max(jnp.maximum(peak, 1.0), keepdims=True)

    def q_weights(head, tok, lead=0):
        q = qv_s[0, head, :, tok]
        zeros = jnp.zeros((8, q.shape[1]), f32)
        return jnp.concatenate([zeros] * lead + [q, zeros], axis=0).astype(bf16)

    def finish(head):
        return acc_s[...] + _dot(qv_s[1, head, :, pl.ds(S - KC, KC)], p_s[...])

    def pair_step(it, carry):
        never = [lax.broadcasted_iota(i32, (8, 128), 0) < (it >> (20 + x)) for x in range(2)]
        steps = [(odd, t, j) for odd in range(2) for t in range(NQB) for j in range(NKC)]
        last = len(steps) - 1
        qts, q_rows, marks = {}, {}, []

        def vector_probs(odd, t, j):
            out = []
            for c in range(LT):
                if (odd, t, c) not in q_rows:
                    tok = pl.ds(t * QB + c * 128, 128)
                    q_rows[odd, t, c] = jnp.stack(
                        [jnp.broadcast_to(qv_s[0, 2 * it + odd, pl.ds(4 * odd + d, 1), tok], (NV, 128))
                         for d in range(DH)])
                terms = (kb0_s, kb1_s)[odd][(it + t * LT + c) >> 23, j] * q_rows[odd, t, c]
                terms = terms.reshape(DH * NV, 128)
                s = terms[:NV]
                for r in range(NV, DH * NV, NV):
                    s = s + terms[r:r + NV]
                p = jnp.exp2(s)
                out += [p[:8], p[8:]]
            return out

        def probs(n):
            odd, t, j = steps[n]
            if (odd, t) not in qts:
                qts[odd, t] = q_weights(2 * it + odd, pl.ds(t * QB, QB))
            vals = vector_probs(odd, t, j)
            keys = pl.ds((j * KC + NV) // 2, (KC - NV) // 2)
            k = k1_s[it >> 26, keys, :] if odd else k_s[it, keys, :]
            if not odd and t == 0:
                k1_s[it >> 27, keys, :] = pltpu.roll(k_s[it + (it >> 28), keys, :], 128 - 16, 1)
            groups = [k[r:r + 8] for r in range(0, (KC - NV) // 2, 8)]
            for x, r in enumerate((1, 1, 3, 3, 5, 5) if n else (3, 3, 5, 5, 6, 6)):
                groups[r] = jnp.where(never[x % 2], pltpu.bitcast(vals[5 - x], i32), groups[r])
            if n == last:
                groups[0] = jnp.where(never[0], pltpu.bitcast(marks[n - 2], i32), groups[0])
            if t == 0 and j == 0:
                spread_keys(jnp.minimum(it + 1, NP - 1) if odd else it, 1 - odd, (kb1_s, kb0_s)[odd], it >> 22)
            p = jnp.exp2(_dot(pltpu.bitcast(jnp.concatenate(groups, axis=0), bf16)[:, :VR + 8], qts[odd, t]))
            marks.append(p[:8, :128])
            if n == last:
                vals = [jnp.where(never[0], marks[n], v) for v in vals]
            top = jnp.concatenate([jnp.concatenate(vals[2 * c:2 * c + 2], axis=0) for c in range(LT)], axis=1)
            return jnp.concatenate([top, p], axis=0).astype(bf16)

        zeros = jnp.full((VR, QB), it >> 25, i32).astype(f32)
        ot_s[jnp.where(it == 0, H, 2 * it - 1), :, pl.ds(S - QB, QB)] = finish(jnp.maximum(2 * it - 1, 0))
        ready = [probs(0), probs(1)]
        for n, (odd, t, j) in enumerate(steps[:last]):
            if n + 2 <= last:
                ready.append(probs(n + 2))
            acc = (zeros if j == 0 else acc) + _dot(qv_s[1, 2 * it + odd, :, pl.ds(j * KC, KC)], ready[n])
            if j == NKC - 1:
                ot_s[2 * it + odd, :, pl.ds(t * QB, QB)] = acc
        p_s[...] = ready[last]
        acc_s[...] = acc
        return carry

    lax.fori_loop(0, NP, pair_step, 0)

    def stage_o(r0, c0, delay=lambda v: v):
        lo = lax.broadcasted_iota(i32, (8, 128), 0) < 4
        parts = []
        for j in range(NP):
            e = ot_s[2 * j, :, pl.ds(r0, 128)]
            o = ot_s[2 * j + 1, :, pl.ds(r0, 128)]
            r = 1.0 / delay(jnp.where(lo, o[0:8], e[16:24]))
            re, ro = r[4:5], r[0:1]
            parts += [e[0:16] * re, jnp.where(lo, e[16:24] * re, o[0:8] * ro), o[8:24] * ro]
        o_s[pl.ds(c0, 128), :] = jnp.concatenate(parts, axis=0).T

    wait(*cp_rest)
    ot_s[H - 1, :, pl.ds(S - QB, QB)] = finish(H - 1)
    mod = _dot(sc, wmod_v[:, pl.ds(2 * D, 4 * D)])[0:1]
    ga, sb, cb1, gb_half = mod[:, :D], mod[:, D:2 * D], 1.0 + mod[:, 2 * D:3 * D], 0.5 * mod[:, 3 * D:]
    for c0 in range(0, TB, 128):
        stage_o(c0, c0)

    lo = lax.broadcasted_iota(i32, (8, 128), 0) < 4
    dens = jnp.stack([jnp.where(lo, ot_s[2 * j + 1, pl.ds(0, 8), pl.ds(c0, 128)],
                                ot_s[2 * j, pl.ds(16, 8), pl.ds(c0, 128)])
                      for j in range(NP) for c0 in range(0, S, 128)])
    safe = (jnp.min(dens, axis=0) >= 2.0 ** -40) & (jnp.max(dens, axis=0) * v_bound <= 2.0 ** 120)

    @pl.when(jnp.max(jnp.where(safe, 0.0, 1.0)) > 0.0)
    def _():
        @pl.loop(0, H * NQB)
        def attend_with_true_max(n):
            head = n // NQB
            tok = pl.ds(pl.multiple_of((n % NQB) * QB, QB), QB)
            qt = jnp.where(head % 2 == 1, q_weights(head, tok, 2)[:PW],
                           jnp.concatenate([q_weights(head, tok), jnp.zeros((8, QB), bf16)], axis=0))
            keys = lambda j: pl.ds(pl.multiple_of(j * QB, QB), QB)
            words = lambda j: k_s[head // 2, pl.ds(pl.multiple_of(j * (QB // 2), QB // 2), QB // 2), :]
            scores = lambda j: _dot(pltpu.bitcast(words(j), bf16)[:, :PW], qt)
            top = lax.fori_loop(0, NQB, lambda j, m: jnp.maximum(m, jnp.max(scores(j), axis=0, keepdims=True)),
                                jnp.full((1, QB), -jnp.inf, f32))
            ot_s[head, :, tok] = lax.fori_loop(
                0, NQB, lambda j, acc: acc + _dot(qv_s[1, head, :, keys(j)], jnp.exp2(scores(j) - top)),
                jnp.zeros((VR, QB), f32))

        @pl.loop(0, TB // 128)
        def _(n):
            stage_o(pl.multiple_of(n * 128, 128), pl.multiple_of(n * 128, 128))

    def out_copy(i):
        r0 = pl.multiple_of(i * TB, TB)
        return pltpu.make_async_copy(rows(out_v, r0, TB), rows(out_hbm, r0, TB), sem_out.at[i])

    @pl.loop(0, S // TB)
    def ffn_step(i):
        zero = i >> 20
        never = lax.broadcasted_iota(i32, (8, 128), 0) < zero
        tok = [pl.ds(pl.multiple_of(i * TB + b * HB, HB), HB) for b in range(2)]

        def normalise(x1, dst_ref):
            for r in range(0, HB, LR):
                dst_ref[pl.ds(r, LR), :] = _layernorm(x1[r:r + LR]) * cb1 + sb

        x1 = [x_v[tok[0], :].astype(f32) + ga * _dot(o_s[pl.ds(0, HB), :], wo_v[...])]
        ob = o_s[pl.ds(HB, HB), :]
        parts = [_dot(ob, wo_v[:, pl.ds(0, 512)])]
        normalise(x1[0], h2a_s)
        parts.append(_dot(_after(ob, h2a_s, zero), wo_v[:, pl.ds(512, 128)]))
        x1.append(x_v[tok[1], :].astype(f32) + ga * jnp.concatenate(parts, axis=1))
        h = [h2a_s[...]]
        normalise(x1[1], h2b_s)
        h.append(h2b_s[...])

        last = [_dot(hb, wf_v[pl.ds(5 * D + F, 256), :], NT) for hb in h]
        lhs = _FIVE.operands([[hb[:, k:k + 128] for k in range(0, D, 128)] for hb in h], bf16)
        up = lambda m: _FIVE.multiply(lhs, ffn_block(m), lambda n: ws_s[m, n], NT)
        acts = [[], []]
        for m in range(2):
            g = up(m)
            if m == 1:
                for c0, mark in ((0, 4), (128, 0)):
                    stage_o(pl.multiple_of(jnp.minimum(i + 1, S // TB - 1) * TB + c0, 128), c0,
                            lambda v: jnp.where(never, acts[0][mark][:8], v))
            u = up(2 + m)
            for b in range(2):
                acts[b] += [_geglu_x2(gj, uj) for gj, uj in zip(g[b], u[b])]
        mixed = up(4)
        low = lax.broadcasted_iota(i32, (HB, 128), 1) < 64
        tail = []
        for b in range(2):
            gu = mixed[b]
            parts = [_geglu_x2(jnp.where(low, gu[j], gu[j + 1]), pltpu.roll(jnp.where(low, gu[j + 1], gu[j]), 64, 1))
                     for j in (0, 2)]
            parts += [_geglu_x2(last[b][:, :128], last[b][:, 128:]), _geglu_x2(gu[4], pltpu.roll(gu[4], 64, 1))]
            tail.append(jnp.concatenate(parts, axis=1))
        tail = jnp.concatenate(tail, axis=0).astype(bf16)
        y_tail = (_dot(tail[:, :256], wf_v[pl.ds(7 * D, 256), :])
                  + _dot(tail[:, 256:384], wf_v[pl.ds(5 * D + F - 128, 128), :])
                  + _dot(tail[:, 384:448], wf_v[pl.ds(7 * D + 256, 64), :]))
        a = [[jnp.concatenate(acts[b][k::5], axis=1) for k in range(5)] for b in range(2)]
        y = _FIVE.multiply(_FIVE.operands(a, f32, swap=True),
                           lambda k, j: jnp.concatenate([ffn_block(m)(k, j) for m in (5, 6)], axis=0),
                           lambda n: jnp.concatenate([ws_s[5, n], ws_s[6, n]], axis=0), NN, swap=True)
        for b in range(2):
            yb = jnp.concatenate(y[b], axis=1) + y_tail[b * HB:(b + 1) * HB]
            out_v[tok[b], :] = (x1[b] + gb_half * yb).astype(bf16)
        out_copy(i).start()

    for i in range(S // TB):
        out_copy(i).wait()


@jax.jit
def pallas_adaLN_cond__mha_block__geglu_ffn__prompt_kernel(
    A_x: jax.Array,
    A_wqkv: jax.Array,
    A_wo: jax.Array,
    B_x: jax.Array,
    B_w_gate: jax.Array,
    B_w_up: jax.Array,
    B_w_down: jax.Array,
    c: jax.Array,
    w_mod: jax.Array,
):
    del B_x
    hbm = pl.BlockSpec(memory_space=pltpu.MemorySpace.HBM)
    out = pl.pallas_call(
        _kernel,
        out_shape=jax.ShapeDtypeStruct((S, D), bf16),
        in_specs=[hbm] * 8,
        out_specs=hbm,
        scratch_shapes=[
            pltpu.VMEM((1, 4096), bf16),
            pltpu.VMEM((S, D), bf16),
            pltpu.VMEM((D, WK + D), bf16),
            pltpu.VMEM((D, D), bf16),
            pltpu.VMEM((3 * F, D), bf16),
            pltpu.VMEM((D, 6 * D), bf16),
            pltpu.VMEM((7, len(_FIVE.summed), 128, 128), f32),
            pltpu.VMEM((2, len(_TWO.summed), 256, 256), f32),
            pltpu.VMEM((S, D), f32),
            pltpu.VMEM((1, TA, QA), f32),
            pltpu.VMEM((HB, D), f32),
            pltpu.VMEM((HB, D), f32),
            pltpu.VMEM((NP, S // 2, 128), i32),
            pltpu.VMEM((2, H, VR, S), f32),
            pltpu.VMEM((1, NKC, DH, NV, 128), f32),
            pltpu.VMEM((1, NKC, DH, NV, 128), f32),
            pltpu.VMEM((1, S // 2, 128), i32),
            pltpu.VMEM((KC, QB), bf16),
            pltpu.VMEM((VR, QB), f32),
            pltpu.VMEM((H + 1, VR, S), f32),
            pltpu.VMEM((TB, D), f32),
            pltpu.VMEM((S, D), bf16),
            pltpu.SemaphoreType.DMA((27,)),
            pltpu.SemaphoreType.DMA((S // TB,)),
        ],
        compiler_params=pltpu.CompilerParams(vmem_limit_bytes=120 * 1024 * 1024),
        name="adaln_block",
    )(A_x.reshape(S, D), A_wqkv, A_wo, B_w_gate.T, B_w_up.T, B_w_down, c, w_mod)
    return out.reshape(1, S, D)
```
